```python
import os as _os
_os.environ.setdefault('JAX_PLATFORMS', 'cpu')
import jax
import jax.numpy as jnp

def _softmax(x, axis=-1):
    return jax.nn.softmax(x, axis=axis)

def _gelu(x):
    return jax.nn.gelu(x, approximate=True)

def _silu(x):
    return jax.nn.silu(x)

def _sigmoid(x):
    return jax.nn.sigmoid(x)

def _layernorm(x, axis=-1, eps=1e-05):
    m = jnp.mean(x, axis=axis, keepdims=True)
    v = jnp.var(x, axis=axis, keepdims=True)
    return (x - m) / jnp.sqrt(v + eps)

def _scatter_add(tgt, idx, src, axis=0):
    return tgt.at[idx].add(src)

def _segment_sum(src, seg, n):
    return jax.ops.segment_sum(src, seg, n)

class _Rng:

    def __init__(self, key):
        self._k = key

    def _next(self):
        self._k, sub = jax.random.split(self._k)
        return sub

    def normal(self, shape):
        return jax.random.normal(self._next(), shape, dtype=jnp.bfloat16)

    def randint(self, lo, hi, shape):
        return jax.random.randint(self._next(), shape, lo, hi, dtype=jnp.int32)

    def uniform(self, shape, lo=0.0, hi=1.0):
        return jax.random.uniform(self._next(), shape, jnp.bfloat16, lo, hi)

    def permutation(self, n):
        return jax.random.permutation(self._next(), n)
kernel_name = 'adaLN_cond__sliding_local_dilated__mixer_channel_mlp__prompt'

def setup_inputs():
    _rng = _Rng(jax.random.key(int.from_bytes(__import__("os").urandom(4), "little")))
    _w = lambda a: (lambda t: t.astype(jnp.bfloat16) if jnp.issubdtype(t.dtype, jnp.floating) else t)(jnp.asarray(a))

    def _A_setup():
        B, S, D = (1, 2048, 512)
        return {'x': _w((lambda *s: _rng.normal(s) * 0.05)(B, S, D)), 'wqkv': _w((lambda *s: _rng.normal(s) * 0.05)(D, 3 * D)), 'wo': _w((lambda *s: _rng.normal(s) * 0.05)(D, D))}
    _A_in = _A_setup()

    def _B_setup():
        B, S, D, F = (1, 2048, 512, 1792)
        return {'x': _w((lambda *s: _rng.normal(s) * 0.05)(B, S, D)), 'w1': _w((lambda *s: _rng.normal(s) * 0.8)(D, F) * D ** (-0.5)), 'b1': _w((lambda *s: _rng.normal(s) * 0.8)(F)), 'w2': _w((lambda *s: _rng.normal(s) * 0.8)(F, D) * F ** (-0.5)), 'b2': _w((lambda *s: _rng.normal(s) * 0.4)(D))}
    _B_in = _B_setup()
    return {'A_x': _A_in['x'], 'A_wqkv': _A_in['wqkv'], 'A_wo': _A_in['wo'], 'B_x': _B_in['x'], 'B_w1': _B_in['w1'], 'B_b1': _B_in['b1'], 'B_w2': _B_in['w2'], 'B_b2': _B_in['b2'], 'c': _w((lambda *s: _rng.normal(s) * 0.05)(1, 512) * 8.0), 'w_mod': _w((lambda *s: _rng.normal(s) * 0.05)(512, 6 * 512) * 512 ** (-0.5) * 8.0)}

def reference(A_x, A_wqkv, A_wo, B_x, B_w1, B_b1, B_w2, B_b2, c, w_mod):

    def _A_ref(x, wqkv, wo):
        B, S, D = x.shape
        H = 32
        Dh = D // H
        W, dil = (8, 2)
        qkv = (lambda x, *d: x.transpose(*d))((x @ wqkv).reshape(B, S, 3, H, Dh), 2, 0, 3, 1, 4)
        q, k, v = (qkv[0], qkv[1], qkv[2])
        scale = Dh ** (-0.5)
        pos = jnp.arange(S)
        off = jnp.arange(W) * dil
        idx = pos[:, None] - off[None, :]
        mask = idx >= 0
        idx_c = jnp.where(mask, idx, 0).reshape(-1)
        kg = k[:, :, idx_c, :].reshape(B, H, S, W, Dh)
        vg = v[:, :, idx_c, :].reshape(B, H, S, W, Dh)
        logits = jnp.einsum('bhsd,bhswd->bhsw', q, kg) * scale
        logits = jnp.where(mask[None, None, :, :], logits, -1000000000.0)
        attn = _softmax(logits, axis=-1)
        o = jnp.einsum('bhsw,bhswd->bhsd', attn, vg)
        return (lambda x, *d: x.transpose(*d))(o, 0, 2, 1, 3).reshape(B, S, D) @ wo

    def _B_ref(x, w1, b1, w2, b2):
        y = _layernorm(x, axis=-1)
        h = _gelu(jnp.einsum('bsd,df->bsf', y, w1) + b1)
        return jnp.einsum('bsf,fd->bsd', h, w2) + b2
    x = A_x
    mod = (_silu(c) @ w_mod).reshape(c.shape[0], 6, 1, -1)
    sa, ca, ga, sb, cb, gb = (mod[:, 0].copy(), mod[:, 1].copy(), mod[:, 2].copy(), mod[:, 3].copy(), mod[:, 4].copy(), mod[:, 5].copy())
    h = _layernorm(x, axis=-1) * (1 + ca) + sa
    x = x + ga * _A_ref(h, A_wqkv, A_wo)
    h = _layernorm(x, axis=-1) * (1 + cb) + sb
    x = x + gb * _B_ref(h, B_w1, B_b1, B_w2, B_b2)
    return x
```

```python
import functools
import contextlib
import jax
import jax.numpy as jnp
from jax import lax
import jax.experimental.pallas as pl
import jax.experimental.pallas.tpu as pltpu

S, D, F = 2048, 512, 1792
H, DH, W, DIL = 32, 16, 8, 2
HALO = 16
LOG2E = 1.4426950408889634
EPS = 1e-5
GC0 = 0.7978845608028654
GC1 = 0.7978845608028654 * 0.044715
f32 = jnp.float32
bf16 = jnp.bfloat16
P = functools.partial


def _ln(x):
    m = jnp.mean(x, axis=-1, keepdims=True)
    xc = x - m
    v = jnp.mean(xc * xc, axis=-1, keepdims=True)
    return xc * lax.rsqrt(v + EPS)


def make(TM=256, RC=8, LC=32, L1C=32, wa=10, wb=20, scopes=0, endw=25, LA=700, L1=500, L23=900):
    NB = S // TM
    assert NB == 8
    KR = TM + HALO
    QB = 4 * KR
    TB = QB + 4 * TM
    NROWS = TB + 8
    NT = TM // 8
    FCH = [(0, 512), (512, 1024), (1024, 1536), (1536, 1792)]
    names = ['tix', 'c', 'wq', 'wk', 'wv', 'wma', 'wo', 'wga', 'wsc', 'w1', 'w2', 'wgb', 'b1', 'b2'] + ['x%d' % b for b in range(NB)]
    SID = {n: i for i, n in enumerate(names)}

    def SC(n):
        return jax.named_scope(n) if scopes else contextlib.nullcontext()

    def kernel(x_hbm, wqkv_hbm, wo_hbm, w1_hbm, b1_hbm, w2_hbm, b2_hbm, c_hbm, wmod_hbm,
               out_hbm, *scr):
        scr = list(scr)
        xb = [scr.pop(0) for _ in range(NB)]
        qkb = [scr.pop(0) for _ in range(NB)]
        x1b = [scr.pop(0) for _ in range(NB)]
        (out_v, wqkv_v, wqkv_p, wo_v, wo_f, wo_p, w1_v, w2_v, wmod_v, b1_v, b2_v, c_v,
         mod_ref, v_scr, ha_v, tix_v, tix2, sems, osems) = scr

        def ocopy(b):
            return pltpu.make_async_copy(out_v.at[pl.ds(b * TM, TM), :], out_hbm.at[0, pl.ds(b * TM, TM), :], osems.at[b])

        def mk(name, src, dst):
            return pltpu.make_async_copy(src, dst, sems.at[SID[name]])

        def wm(lo, hi, name):
            return mk(name, wmod_hbm.at[:, lo * D:hi * D], wmod_v.at[:, lo * D:hi * D])

        cp = dict(
            c=mk('c', c_hbm, c_v),
            wq=mk('wq', wqkv_hbm.at[:, 0:D], wqkv_v.at[:, 0:D]),
            wk=mk('wk', wqkv_hbm.at[:, D:2 * D], wqkv_v.at[:, D:2 * D]),
            wv=mk('wv', wqkv_hbm.at[:, 2 * D:3 * D], wqkv_v.at[:, 2 * D:3 * D]),
            wma=wm(0, 2, 'wma'), wga=wm(2, 3, 'wga'), wsc=wm(3, 5, 'wsc'), wgb=wm(5, 6, 'wgb'),
            wo=mk('wo', wo_hbm, wo_v.at[pl.ds(0, D), :]),
            w1=mk('w1', w1_hbm, w1_v), w2=mk('w2', w2_hbm, w2_v),
            b1=mk('b1', b1_hbm, b1_v), b2=mk('b2', b2_hbm, b2_v),
        )
        for b in range(NB):
            cp['x%d' % b] = mk('x%d' % b, x_hbm.at[0, pl.ds(b * TM, TM), :], xb[b].at[pl.ds(0, TM), :])
        order = ['c', 'x0', 'wma', 'x1', 'wq', 'wk', 'wv', 'x2', 'wo', 'wga', 'wsc', 'x3', 'x4', 'x5', 'b1', 'w1',
                 'w2', 'wgb', 'b2', 'x6', 'x7']
        with SC('start'):
            for o in order:
                cp[o].start()

        def wait(*ns):
            with SC('w_' + ns[0]):
                for n in ns:
                    cp[n].wait()

        lane0 = lax.broadcasted_iota(jnp.int32, (8, 128), 1)
        tix_v[...] = jnp.where(lane0 == 0, TB, jnp.where(lane0 == 1, TM, jnp.where(lane0 == 2, 0, D)))
        cp_tix = pltpu.make_async_copy(tix_v, tix2, sems.at[SID['tix']])
        cp_tix.start()
        tix = [None] * 4

        def silu_c():
            c = c_v[...].astype(f32)
            sc = c * jax.nn.sigmoid(c)
            return jnp.broadcast_to(sc, (8, D)).astype(bf16)

        def mod_part(lo, hi):
            mod_ref[:, lo * D:hi * D] = jnp.dot(silu_c(), wmod_v[:, lo * D:hi * D], preferred_element_type=f32)

        def modv(i):
            return mod_ref[0:1, i * D:(i + 1) * D]

        def perm_part(t):
            lane = lax.broadcasted_iota(jnp.int32, (D // 2, 128), 1)
            e = (lane >> 2) & 3
            r = lax.broadcasted_iota(jnp.int32, (128, 128), 0)
            cc = lax.broadcasted_iota(jnp.int32, (128, 128), 1)
            ch = [pltpu.bitcast(wqkv_v[:, t * D + 128 * c:t * D + 128 * (c + 1)], jnp.uint32) for c in range(4)]
            for cpi in range(4):
                tgt = ((r & 3) << 5) | (((cpi ^ ((r >> 2) & 3))) << 3) | (r >> 4)
                Qm = jnp.where(cc == tgt, 1.0, 0.0).astype(bf16)
                mg = ch[cpi ^ 0]
                for ee in range(1, 4):
                    mg = jnp.where(e == ee, ch[cpi ^ ee], mg)
                mg = pltpu.bitcast(mg, bf16)
                wqkv_p[:, t * D + 128 * cpi:t * D + 128 * (cpi + 1)] = jnp.dot(
                    mg, Qm, preferred_element_type=f32).astype(bf16)

        def dynrows(r, n):
            return pl.ds(pl.multiple_of(tix[2] + r, min(n, 16)), n)

        def tok16(tokv):
            return jnp.concatenate([tokv, tokv], axis=0).astype(bf16)

        def permwo_chunk(n, tokv):
            if tokv is not None:
                wo_v[pl.ds(pl.multiple_of(tix[3], 16), 16), 0:128] = tok16(tokv)
            wo_f[n] = wo_v[0:D, 128 * n:128 * (n + 1)].astype(f32)
            for cpi in range(4):
                for t in range(4):
                    parts = []
                    for g in range(4):
                        d = ((cpi ^ g) << 2) | t
                        parts.append(wo_f[n, pl.ds(g * 128 + d, 8, stride=16), :])
                    wo_p[cpi * 128 + t * 32:cpi * 128 + t * 32 + 32, 128 * n:128 * (n + 1)] = (
                        jnp.concatenate(parts, axis=0).astype(bf16))

        def ln1_chunk(b, j, tokv):
            r0 = j * L1C
            if tokv is not None:
                xb[b][pl.ds(pl.multiple_of(tix[1], 16), 16), 0:128] = tok16(tokv)
            x = xb[b][r0:r0 + L1C, :].astype(f32)
            hc = (_ln(x) * (1.0 + modv(1)) + modv(0)).astype(bf16)
            ha_v[dynrows(S + b * TM + r0, L1C), :] = hc

        def ln23_chunk(b, j, tokv):
            r0 = j * LC
            if tokv is not None:
                x1b[b][pl.ds(pl.multiple_of(tix[1], 8), 8), 0:128] = tokv
            x1 = x1b[b][r0:r0 + LC, :]
            h2 = _ln(x1) * (1.0 + modv(4)) + modv(3)
            yc = _ln(h2).astype(bf16)
            ha_v[dynrows(2 * S + b * TM + r0, LC), :] = yc

        def attn_chunk(b, j, tokv):
            r0 = j * RC
            qk = qkb[b]
            if tokv is not None:
                qk[pl.ds(pl.multiple_of(tix[0], 8), 8), :] = tokv
            q = [qk[QB + c * TM + r0:QB + c * TM + r0 + RC, :] for c in range(4)]
            logits = []
            for w in range(W):
                off = HALO + r0 - DIL * w
                acc = None
                for c in range(4):
                    p = q[c] * qk[pl.ds(c * KR + off, RC), :]
                    acc = p if acc is None else acc + p
                acc = acc + pltpu.roll(acc, 64, 1)
                acc = acc + pltpu.roll(acc, 32, 1)
                if b == 0 and r0 < DIL * w:
                    row = r0 + lax.broadcasted_iota(jnp.int32, (RC, 128), 0)
                    acc = jnp.where(row >= DIL * w, acc, -1e9 * LOG2E)
                logits.append(acc)
            m = logits[0]
            for w in range(1, W):
                m = jnp.maximum(m, logits[w])
            ps = [jnp.exp2(l - m) for l in logits]
            den = ps[0]
            for w in range(1, W):
                den = den + ps[w]
            inv = 1.0 / den
            outs = []
            for c in range(4):
                acc = None
                for w in range(W):
                    off = HALO + b * TM + r0 - DIL * w
                    t = ps[w] * v_scr[c, pl.ds(off, RC), :]
                    acc = t if acc is None else acc + t
                outs.append(acc * inv)
            ha_v[dynrows(b * TM + r0, RC), :] = jnp.concatenate(outs, axis=1).astype(bf16)

        def attn_fns(b):
            return [P(attn_chunk, b, j) for j in range(TM // RC)]

        def ln1_fns(b):
            return [P(ln1_chunk, b, j) for j in range(TM // L1C)]

        def ln23_fns(b):
            return [P(ln23_chunk, b, j) for j in range(TM // LC)]

        def permwo_fns():
            return [P(permwo_chunk, n) for n in range(4)]

        hs = {}

        def pQ(b, t, dl):
            if dl or b not in hs:
                hs[b] = ha_v[S + b * TM:S + (b + 1) * TM, :]
            r = jnp.dot(hs[b], wqkv_p[:, t * D:(t + 1) * D], preferred_element_type=f32)
            qk = qkb[b]
            for c in range(4):
                rc = r[:, 128 * c:128 * (c + 1)]
                if t == 0:
                    qk[QB + c * TM:QB + (c + 1) * TM, :] = rc * (DH ** -0.5 * LOG2E)
                elif t == 1:
                    qk[c * KR + HALO:(c + 1) * KR, :] = rc
                    if b + 1 < NB:
                        qkb[b + 1][c * KR:c * KR + HALO, :] = rc[TM - HALO:TM, :]
                else:
                    v_scr[c, HALO + b * TM:HALO + (b + 1) * TM, :] = rc
            return r

        def pW(b):
            a = jnp.dot(ha_v[b * TM:(b + 1) * TM, :], wo_p[...], preferred_element_type=f32)
            x1b[b][0:TM, :] = xb[b][0:TM, :].astype(f32) + modv(2) * a
            return a

        st = {}

        def p1(b, j):
            if j == 0:
                st[b] = dict(y=ha_v[2 * S + b * TM:2 * S + (b + 1) * TM, :], g={}, z=None)
            lo, hi = FCH[j]
            b1 = b1_v[...].astype(f32).reshape(1, F)
            u = jnp.dot(st[b]['y'], w1_v[:, lo:hi], preferred_element_type=f32) + b1[:, lo:hi]
            t = jnp.tanh(u * (GC0 + GC1 * (u * u)))
            st[b]['g'][j] = (u + u * t).astype(bf16)
            return u

        def p2(b, j):
            lo, hi = FCH[j]
            zp = jnp.dot(st[b]['g'][j], w2_v[lo:hi, :], preferred_element_type=f32)
            st[b]['z'] = zp if st[b]['z'] is None else st[b]['z'] + zp
            if j == 3:
                gb = modv(5)
                out_v[b * TM:(b + 1) * TM, :] = (
                    x1b[b][0:TM, :] + (0.5 * gb) * st[b]['z'] + gb * b2_v[...].astype(f32).reshape(1, D)).astype(bf16)
                ocopy(b).start()
            return zp

        def dur(pc):
            k = pc[0]
            if k in ('q', 'w'):
                return 4 * TM
            if k == 'm1' or k == 'm2':
                lo, hi = FCH[pc[2]]
                return (hi - lo) // 128 * TM
            return 0

        def run_piece(pc):
            k = pc[0]
            if k == 'q':
                return pQ(pc[1], pc[2], len(pc) > 3)
            if k == 'w':
                return pW(pc[1])
            if k == 'm1':
                return p1(pc[1], pc[2])
            if k == 'm2':
                return p2(pc[1], pc[2])
            if k == 'perm':
                perm_part(pc[1])
            elif k == 'mod':
                mod_part(pc[1], pc[2])
            elif k == 'wait':
                wait(*pc[1:])
            return None

        def run_seq(pieces, groups):
            t0s = []
            t = 0
            for pc in pieces:
                t0s.append(t)
                t += dur(pc)
            t0s.append(t)
            sched = {i: [] for i in range(len(pieces))}
            G = 8
            seen = set()
            dlf = []
            for i, pc in enumerate(pieces):
                d = pc[0] in ('wait', 'w') or (pc[0] == 'm1' and pc[2] == 0)
                if pc[0] == 'q':
                    if pc[1] not in seen:
                        d = True
                        seen.add(pc[1])
                    elif i + 1 < len(pieces) and pieces[i + 1][0] == 'wait':
                        d = True
                        pieces[i] = pc + ('dl',)
                dlf.append(d)

            def is_dl(i):
                return dlf[i]
            for fns, i0, i1, lat in groups:
                dls = [t0s[i] for i in range(i0 + 1, i1 + 1) if is_dl(i)] + [t0s[i1 + 1]]
                slots = []
                for i in range(i0, i1 + 1):
                    if i + 1 < len(pieces) and pieces[i + 1][0] == 'wait':
                        continue
                    wt = wa if pieces[i][0] == 'm1' else wb
                    for tt in range(t0s[i], t0s[i + 1], G):
                        if any(d - lat <= tt < d for d in dls):
                            continue
                        slots.append((i, tt, wt))
                tot = sum(s_[2] for s_ in slots)
                n = len(fns)
                acc = 0
                kk = 0
                for (i, tt, wt) in slots:
                    while kk < n and kk / n * tot < acc + wt:
                        sched[i].append(((tt - t0s[i]) / dur(pieces[i]), kk, fns[kk]))
                        kk += 1
                    acc += wt
                assert kk == n
            for i, pc in enumerate(pieces):
                arr = run_piece(pc)
                for fr, _, fn in sorted(sched[i], key=lambda t_: (t_[0], t_[1])):
                    ntl = arr.shape[1] // 128 * NT
                    ti = min(int(fr * ntl), ntl - 1)
                    n, r = divmod(ti, NT)
                    fn(arr[8 * r:8 * r + 8, 128 * n:128 * (n + 1)])

        def Qs(b):
            return [('q', b, 0), ('q', b, 1), ('q', b, 2)]

        def Ms(b):
            return [('m1', b, 0), ('m1', b, 1), ('m2', b, 0), ('m1', b, 2), ('m2', b, 1), ('m1', b, 3), ('m2', b, 2), ('m2', b, 3)]

        for c in range(4):
            qkb[0][c * KR:c * KR + HALO, :] = jnp.zeros((HALO, 128), f32)
        v_scr[:, 0:HALO, :] = jnp.zeros((4, HALO, 128), f32)
        cp_tix.wait()
        for i in range(4):
            tix[i] = tix2[0, i]
        wait('c', 'x0', 'wma', 'x1')
        with SC('ln1_01'):
            mod_part(0, 2)
            for fn in ln1_fns(0) + ln1_fns(1):
                fn(None)
        ew = endw / 100.0
        pieces = []
        groups = []

        def add(*pcs):
            i0 = len(pieces)
            pieces.extend(pcs)
            return i0, len(pieces) - 1

        ix = {}

        def addn(*pcs):
            for pc in pcs:
                ix[pc] = len(pieces)
                pieces.append(pc)

        def grp(fns, a, b_, lat):
            groups.append((fns, ix[a], ix[b_], lat))

        addn(('wait', 'wq'), ('perm', 0), ('q', 0, 0), ('q', 1, 0))
        addn(('wait', 'wk', 'wv', 'x2'), ('perm', 1), ('q', 0, 1), ('perm', 2), ('q', 0, 2), ('q', 1, 1), ('q', 1, 2),
             ('q', 2, 0), ('q', 2, 1))
        addn(('wait', 'wo', 'wga', 'wsc', 'x3', 'x4', 'x5'), ('mod', 2, 5), ('q', 2, 2), ('w', 0), *Qs(3), *Qs(4), ('w', 1), *Qs(5))
        addn(('wait', 'b1', 'w1', 'w2', 'wgb', 'b2', 'x6', 'x7'), ('mod', 5, 6), *Ms(0))
        addn(('w', 2), *Qs(6), *Ms(1), ('w', 3), *Qs(7), *Ms(2))
        for b in (3, 4, 5, 6):
            addn(('w', b + 1), *Ms(b))
        addn(*Ms(7))
        grp(ln1_fns(2), ('q', 0, 1), ('q', 1, 2), L1)
        grp(attn_fns(0), ('q', 1, 1), ('q', 2, 1), LA)
        grp(permwo_fns(), ('q', 2, 2), ('q', 2, 2), 500)
        grp(ln1_fns(3), ('q', 2, 2), ('w', 0), L1)
        grp(ln23_fns(0), ('q', 3, 0), ('q', 4, 2), L23)
        grp(ln1_fns(4), ('q', 3, 0), ('q', 3, 2), L1)
        grp(attn_fns(1), ('w', 0), ('q', 4, 2), LA)
        grp(ln1_fns(5), ('q', 4, 0), ('w', 1), L1)
        grp(ln23_fns(1), ('q', 5, 0), ('m2', 0, 3), L23)
        grp(attn_fns(2), ('w', 1), ('m2', 0, 3), LA)
        grp(ln1_fns(6), ('m1', 0, 0), ('m2', 0, 3), L1)
        grp(ln23_fns(2), ('q', 6, 0), ('q', 6, 2), L23)
        grp(attn_fns(3), ('m1', 1, 0), ('m2', 1, 3), LA)
        grp(ln1_fns(7), ('m1', 1, 0), ('m2', 1, 3), L1)
        grp(ln23_fns(3), ('q', 7, 0), ('q', 7, 2), L23)
        grp(attn_fns(4), ('m1', 2, 0), ('m2', 2, 3), LA)
        for b in (3, 4, 5, 6):
            grp(ln23_fns(b + 1), ('m1', b, 0), ('m2', b, 3), L23)
            if b + 2 < NB:
                grp(attn_fns(b + 2), ('m1', b, 0), ('m2', b, 3), LA)
        run_seq(pieces, groups)
        for b in range(NB):
            ocopy(b).wait()

    def fn(A_x, A_wqkv, A_wo, B_x, B_w1, B_b1, B_w2, B_b2, c, w_mod):
        anyspec = pl.BlockSpec(memory_space=pl.ANY)
        return pl.pallas_call(
            kernel,
            in_specs=[anyspec] * 9,
            out_specs=anyspec,
            out_shape=jax.ShapeDtypeStruct((1, S, D), bf16),
            scratch_shapes=(
                [pltpu.VMEM((TM + 16, D), bf16) for _ in range(NB)]
                + [pltpu.VMEM((NROWS, 128), f32) for _ in range(NB)]
                + [pltpu.VMEM((TM + 8, D), f32) for _ in range(NB)]
                + [
                pltpu.VMEM((S, D), bf16),
                pltpu.VMEM((D, 3 * D), bf16),
                pltpu.VMEM((D, 3 * D), bf16),
                pltpu.VMEM((D + 16, D), bf16),
                pltpu.VMEM((4, D, 128), f32),
                pltpu.VMEM((D, D), bf16),
                pltpu.VMEM((D, F), bf16),
                pltpu.VMEM((F, D), bf16),
                pltpu.VMEM((D, 6 * D), bf16),
                pltpu.VMEM((F,), bf16),
                pltpu.VMEM((D,), bf16),
                pltpu.VMEM((1, D), bf16),
                pltpu.VMEM((8, 6 * D), f32),
                pltpu.VMEM((4, S + HALO, 128), f32),
                pltpu.VMEM((3 * S, D), bf16),
                pltpu.VMEM((8, 128), jnp.int32),
                pltpu.SMEM((8, 128), jnp.int32),
                pltpu.SemaphoreType.DMA((len(names),)),
                pltpu.SemaphoreType.DMA((NB,)),
            ]),
            compiler_params=pltpu.CompilerParams(
                vmem_limit_bytes=100 * 1024 * 1024,
            ),
        )(A_x, A_wqkv, A_wo, B_w1, B_b1, B_w2, B_b2, c, w_mod)
    return fn


_impl = make()


@jax.jit
def pallas_adaLN_cond__sliding_local_dilated__mixer_channel_mlp__prompt_kernel(
    A_x: jax.Array,
    A_wqkv: jax.Array,
    A_wo: jax.Array,
    B_x: jax.Array,
    B_w1: jax.Array,
    B_b1: jax.Array,
    B_w2: jax.Array,
    B_b2: jax.Array,
    c: jax.Array,
    w_mod: jax.Array,
):
    return _impl(A_x, A_wqkv, A_wo, B_x, B_w1, B_b1, B_w2, B_b2, c, w_mod)
```

```python
import bisect
import contextlib
import functools

import jax
import jax.numpy as jnp
from jax import lax
import jax.experimental.pallas as pl
import jax.experimental.pallas.tpu as pltpu

S, D, F = 2048, 512, 1792
H, DH, W, DIL = 32, 16, 8, 2
HALO = 16
LOG2E = 1.4426950408889634
EPS = 1e-5
GC0 = 0.7978845608028654
GC1 = 0.7978845608028654 * 0.044715
f32 = jnp.float32
bf16 = jnp.bfloat16
P = functools.partial


def _ln(x):
    m = jnp.mean(x, axis=-1, keepdims=True)
    xc = x - m
    v = jnp.mean(xc * xc, axis=-1, keepdims=True)
    return xc * jnp.exp2(-0.5 * jnp.log2(v + EPS))


def _bc(x, r8):
    R, N = x.shape
    return x.reshape(R // 8, 8, N), r8.reshape(1, 8, N)


def _mul8(x, r8):
    if r8.shape[0] == 1:
        return x * r8
    a, b = _bc(x, r8)
    return (a * b).reshape(x.shape)


def _add8(x, r8):
    if r8.shape[0] == 1:
        return x + r8
    a, b = _bc(x, r8)
    return (a + b).reshape(x.shape)


u32 = jnp.uint32


def _pk(x):
    return pltpu.bitcast(x, u32)


def _upk(x):
    return pltpu.bitcast(x, bf16)


def make(TM=256, RC=8, LC=32, L1C=32, wa=10, wb=20, scopes=0, LA=300, L1=300, L23=300, sa=12, T=250, sb=20,
         D1=350, D23=650, DA=450, LAh=250, mh0=0, mh1=0, tail=1, plan=3, split=1, LP=300, a0x=0, L1h=100, rp=0, fen=0, fpos=50, wre=1, m8=1, xre=0, prio=0, PW=17, xo=0, r2e=0, bm=1, oprio=0):
    NB = S // TM
    assert NB == 8
    KR = TM + HALO
    QB = 4 * KR
    VT = 4 * KR
    TB = QB + 4 * TM
    NROWS = TB + 8
    NT = TM // 8
    FCH = [(0, 512), (512, 1024), (1024, 1536), (1536, 1792)]
    names = ['tix', 'c', 'wq', 'wk', 'wv', 'wma', 'wsa', 'wca', 'wo', 'wga', 'wsc', 'w1', 'w2', 'wgb', 'b1', 'b2'] + ['x%d' % b for b in range(NB)]
    SID = {n: i for i, n in enumerate(names)}

    def SC(n):
        return jax.named_scope(n) if scopes else contextlib.nullcontext()

    def kernel(x_hbm, wqkv_hbm, wo_hbm, w1_hbm, b1_hbm, w2_hbm, b2_hbm, c_hbm, wmod_hbm,
               out_hbm, *scr):
        scr = list(scr)
        xb = [scr.pop(0) for _ in range(NB)]
        qkb = [scr.pop(0) for _ in range(NB)]
        x1b = [scr.pop(0) for _ in range(NB)]
        vb = [scr.pop(0) for _ in range(NB)]
        (out_v, wqkv_v, wqkv_p, wo_v, wo_f, wo_p, w1_v, w2_v, wmod_v, b1_v, b2_v, c_v,
         mod_ref, ha_v, w1_p, w2_p, b1_f, sc_v, sa_v, bias_v, tix_v, tix2, sems, osems) = scr

        wqkv_p = wqkv_p.bitcast(bf16)
        wo_p = wo_p.bitcast(bf16)
        ha_v = ha_v.bitcast(bf16)
        if wre:
            w1_v = w1_p.bitcast(bf16)
            w2_v = w2_p.bitcast(bf16)
        if xre:
            xb = [r_.bitcast(bf16) for r_ in xb]
        ocopies = []

        def ocopy(b, c0, c1):
            cpy = pltpu.make_async_copy(out_v.at[pl.ds(b * TM, TM), pl.ds(128 * c0, 128 * (c1 - c0))],
                                        out_hbm.at[0, pl.ds(b * TM, TM), pl.ds(128 * c0, 128 * (c1 - c0))],
                                        osems.at[len(ocopies)])
            ocopies.append(cpy)
            cpy.start(priority=oprio if b < NB - 1 else 0)

        def mk(name, src, dst):
            return pltpu.make_async_copy(src, dst, sems.at[SID[name]])

        def wm(lo, hi, name):
            return mk(name, wmod_hbm.at[:, lo * D:hi * D], wmod_v.at[:, lo * D:hi * D])

        cp = dict(
            c=mk('c', c_hbm, c_v),
            wq=mk('wq', wqkv_hbm.at[:, 0:D], wqkv_v.at[:, 0:D]),
            wk=mk('wk', wqkv_hbm.at[:, D:2 * D], wqkv_v.at[:, D:2 * D]),
            wv=mk('wv', wqkv_hbm.at[:, 2 * D:3 * D], wqkv_v.at[:, 2 * D:3 * D]),
            **(dict(wsa=wm(0, 1, 'wsa'), wca=wm(1, 2, 'wca')) if plan == 3 else dict(wma=wm(0, 2, 'wma'))), wga=wm(2, 3, 'wga'), wsc=wm(3, 5, 'wsc'), wgb=wm(5, 6, 'wgb'),
            wo=mk('wo', wo_hbm, wo_v.at[pl.ds(0, D), :]),
            w1=mk('w1', w1_hbm, w1_v.at[pl.ds(0, D), :]), w2=mk('w2', w2_hbm, w2_v.at[pl.ds(0, F), :]),
            b1=mk('b1', b1_hbm, b1_v), b2=mk('b2', b2_hbm, b2_v),
        )
        for b in range(NB):
            cp['x%d' % b] = mk('x%d' % b, x_hbm.at[0, pl.ds(b * TM, TM), :], xb[b].at[pl.ds(0, TM), :])
        order = ['c', 'x0', 'wma', 'x1', 'wq', 'wk', 'wv', 'x2', 'x3', 'wo', 'wga', 'wsc', 'x4', 'x5', 'b1', 'w1',
                 'w2', 'wgb', 'b2', 'x6', 'x7']
        if plan == 3:
            order = ['c', 'x0', 'wca', 'wk'] + (['x1', 'wv'] if xo else ['wv', 'x1']) + ['wsa', 'wq'] + order[7:]
        cp = {k_: v_ for k_, v_ in cp.items() if k_ in order}
        with SC('start'):
            for io, o in enumerate(order):
                pr = {0: 0, 1: int(io < 8), 2: io % 2, 3: 1, 4: int(io >= 5), 5: int(io >= 9), 6: int(io >= 15)}[prio]
                cp[o].start(priority=pr)

        def wait(*ns):
            with SC('w_' + ns[0]):
                for n in ns:
                    cp[n].wait()

        TIXV = [TB, TM, 0, D, VT, F, D // 2, F // 2]
        lane0 = lax.broadcasted_iota(jnp.int32, (8, 128), 1)
        tv = jnp.zeros((8, 128), jnp.int32)
        for i, v_ in enumerate(TIXV):
            tv = jnp.where(lane0 == i, v_, tv)
        tix_v[...] = tv
        cp_tix = pltpu.make_async_copy(tix_v, tix2, sems.at[SID['tix']])
        cp_tix.start()
        tix = [None] * len(TIXV)

        def silu_init():
            c = c_v[...].astype(f32)
            sc = c * jax.nn.sigmoid(c)
            sc_v[...] = jnp.broadcast_to(sc, (16, D)).astype(bf16)

        def silu_c():
            return sc_v[0:8, :]

        def mod_tile(n):
            if isinstance(n, tuple):
                nn = n[1]
                bias_v[:, 128 * nn:128 * (nn + 1)] = jnp.dot(sa_v[0:8, :], wqkv_p[0:D, 128 * nn:128 * (nn + 1)],
                                                             preferred_element_type=f32)
                return
            mod_ref[:, 128 * n:128 * (n + 1)] = jnp.dot(silu_c(), wmod_v[:, 128 * n:128 * (n + 1)], preferred_element_type=f32)
            if 4 <= n < 8 or 16 <= n < 20:
                mod_ref[:, 128 * n:128 * (n + 1)] = 1.0 + mod_ref[:, 128 * n:128 * (n + 1)]
            if n < 4 and plan == 3:
                sa8 = mod_ref[:, 128 * n:128 * (n + 1)]
                sa_v[:, 128 * n:128 * (n + 1)] = jnp.concatenate([sa8, sa8], axis=0).astype(bf16)
            if n >= 20:
                gb = mod_ref[:, 128 * n:128 * (n + 1)]
                b2 = b2_v[...].astype(f32).reshape(1, D)[:, 128 * (n - 20):128 * (n - 19)]
                mod_ref[:, 128 * (n + 4):128 * (n + 5)] = gb * b2
                mod_ref[:, 128 * n:128 * (n + 1)] = 0.5 * gb

        MODS = {}

        def dot_mods(lhs_, wget, c0, ncol, mods):
            if not mods:
                return jnp.dot(lhs_, wget(c0, c0 + ncol), preferred_element_type=f32)
            outs = []
            for c in range(ncol // 128):
                outs.append(jnp.dot(lhs_, wget(c0 + 128 * c, c0 + 128 * (c + 1)), preferred_element_type=f32))
                for n in mods[c]:
                    mod_tile(n)
            return jnp.concatenate(outs, axis=1)

        def modv(i):
            return mod_ref[0:(8 if m8 else 1), i * D:(i + 1) * D]

        def perm_part(t):
            lane = lax.broadcasted_iota(jnp.int32, (D // 2, 128), 1)
            e = (lane >> 2) & 3
            r = lax.broadcasted_iota(jnp.int32, (128, 128), 0)
            cc = lax.broadcasted_iota(jnp.int32, (128, 128), 1)
            ch = [pltpu.bitcast(wqkv_v[:, t * D + 128 * c:t * D + 128 * (c + 1)], jnp.uint32) for c in range(4)]
            for cpi in range(4):
                tgt = ((r & 3) << 5) | (((cpi ^ ((r >> 2) & 3))) << 3) | (r >> 4)
                Qm = jnp.where(cc == tgt, 1.0, 0.0).astype(bf16)
                mg = ch[cpi ^ 0]
                for ee in range(1, 4):
                    mg = jnp.where(e == ee, ch[cpi ^ ee], mg)
                mg = pltpu.bitcast(mg, bf16)
                wqkv_p[0:D, t * D + 128 * cpi:t * D + 128 * (cpi + 1)] = jnp.dot(
                    mg, Qm, preferred_element_type=f32).astype(bf16)

        def dynrows(r, n):
            return pl.ds(pl.multiple_of(tix[2] + r, 16), n)

        def tok16(tokv):
            return jnp.concatenate([tokv, tokv], axis=0).astype(bf16)

        def permwo_task(n):
            def sA(tokv):
                if tokv is not None:
                    wo_v[pl.ds(pl.multiple_of(tix[3], 16), 16), 0:128] = tok16(tokv)
                wf = wo_v[0:D, 128 * n:128 * (n + 1)].astype(f32)
                for hh in range(H):
                    wo_f[n, pl.ds(hh * PW, 16), :] = wf[16 * hh:16 * hh + 16, :]
                for cpi in range(4):
                    for t in range(4):
                        parts = []
                        for g in range(4):
                            d = ((cpi ^ g) << 2) | t
                            parts.append(wo_f[n, pl.ds(g * 8 * PW + d, 8, stride=PW), :])
                        wo_p[cpi * 128 + t * 32:cpi * 128 + t * 32 + 32, 128 * n:128 * (n + 1)] = (
                            jnp.concatenate(parts, axis=0).astype(bf16))
            return [(0, sA)]

        def ln1_task(b, j):
            r0 = j * L1C
            stt = {}

            def sA(tokv):
                if tokv is not None:
                    xb[b][pl.ds(pl.multiple_of(tix[1], 16), 16), 0:128] = tok16(tokv)
                x = xb[b][r0:r0 + L1C, :].astype(f32)
                hh = _mul8(_ln(x), modv(1))
                if not (plan == 3 and b < 2):
                    hh = _add8(hh, modv(0))
                stt['h'] = hh.astype(bf16)

            def sB(tokv):
                ha_v[dynrows(S + b * TM + r0, L1C), :] = stt['h']

            return [(0, sA), (D1, sB)]

        def ln23_task(b, j):
            r0 = j * LC
            stt = {}

            def sA(tokv):
                if tokv is not None:
                    x1b[b][pl.ds(pl.multiple_of(tix[1], 8), 8), 0:128] = tokv
                x1 = x1b[b][r0:r0 + LC, :]
                h2 = _add8(_mul8(_ln(x1), modv(4)), modv(3))
                stt['y'] = _ln(h2).astype(bf16)

            def sB(tokv):
                ha_v[dynrows(2 * S + b * TM + r0, LC), :] = stt['y']

            return [(0, sA), (D23, sB)]

        attprev = {}

        def attn_task(b, j, micro):
            r0 = j * RC
            qk = qkb[b]
            stt = dict(logits=[], outs=[])

            def qk_step(w, tokv):
                if tokv is not None:
                    qk[pl.ds(pl.multiple_of(tix[0], 8), 8), :] = tokv
                if w == 0:
                    stt['q'] = [qk[QB + c * TM + r0:QB + c * TM + r0 + RC, :] for c in range(4)]
                q = stt['q']
                off = HALO + r0 - DIL * w
                ps_ = [q[c] * qk[pl.ds(c * KR + off, RC), :] for c in range(4)]
                acc = (ps_[0] + ps_[1]) + (ps_[2] + ps_[3])
                if micro:
                    acc = (acc + pltpu.roll(acc, 64, 1)) + (pltpu.roll(acc, 32, 1) + pltpu.roll(acc, 96, 1))
                else:
                    acc = acc + pltpu.roll(acc, 64, 1)
                    acc = acc + pltpu.roll(acc, 32, 1)
                if b == 0 and r0 < DIL * w:
                    row = r0 + lax.broadcasted_iota(jnp.int32, (RC, 128), 0)
                    acc = jnp.where(row >= DIL * w, acc, -1e9 * LOG2E)
                stt['logits'].append(acc)
                if w == W - 1:
                    lg = stt['logits']
                    m = jnp.maximum(jnp.maximum(jnp.maximum(lg[0], lg[1]), jnp.maximum(lg[2], lg[3])),
                                    jnp.maximum(jnp.maximum(lg[4], lg[5]), jnp.maximum(lg[6], lg[7])))
                    ps = [jnp.exp2(l - m) for l in lg]
                    den = ((ps[0] + ps[1]) + (ps[2] + ps[3])) + ((ps[4] + ps[5]) + (ps[6] + ps[7]))
                    r_ = pl.reciprocal(den, approx=True)
                    stt['inv'] = r_ * (2.0 - den * r_)
                    stt['ps'] = ps

            def pv_step(c, tokv):
                if tokv is not None:
                    vb[b][pl.ds(pl.multiple_of(tix[4], 8), 8), :] = tokv
                ps = stt['ps']
                ts = [ps[w] * vb[b][pl.ds(c * KR + HALO + r0 - DIL * w, RC), :] for w in range(W)]
                acc = ((ts[0] + ts[1]) + (ts[2] + ts[3])) + ((ts[4] + ts[5]) + (ts[6] + ts[7]))
                stt['outs'].append(acc * stt['inv'])
                if c == 3:
                    o = jnp.concatenate(stt['outs'], axis=1)
                    if RC >= 16:
                        ha_v[dynrows(b * TM + r0, RC), :] = o.astype(bf16)
                    elif j % 2 == 0:
                        attprev[b] = o
                    else:
                        oo = jnp.concatenate([attprev[b], o], axis=0).astype(bf16)
                        ha_v[dynrows(b * TM + r0 - RC, 2 * RC), :] = oo

            if micro:
                return [(sa * w, P(qk_step, w)) for w in range(W)] + [(T + sb * c, P(pv_step, c)) for c in range(4)]

            def allA(tokv):
                qk_step(0, tokv)
                for w in range(1, W):
                    qk_step(w, None)
                for c in range(3):
                    pv_step(c, None)

            def allB(tokv):
                pv_step(3, None)
            return [(0, allA), (DA, allB)]

        def fix_task(t, b, c):
            def sA(tokv):
                ref, ti = (qkb[b], 0) if t == 1 else (vb[b], 4)
                if tokv is not None:
                    ref[pl.ds(pl.multiple_of(tix[ti], 8), 8), :] = tokv
                lo = c * KR + (HALO if b == 0 else 0)
                hi = c * KR + (HALO if b == 2 else KR)
                ref[lo:hi, :] = _add8(ref[lo:hi, :], bias_v[:, t * D + 128 * c:t * D + 128 * (c + 1)])
            return [(0, sA)]

        def fix_fns(t):
            return [fix_task(t, b, c) for b in range(3) for c in range(4)]

        def attn_fns(b, mi=1):
            return [attn_task(b, j, mi) for j in range(TM // RC)]

        def ln1_fns(b):
            return [ln1_task(b, j) for j in range(TM // L1C)]

        def ln23_fns(b):
            return [ln23_task(b, j) for j in range(TM // LC)]

        def permwo_fns():
            return [permwo_task(n) for n in range(4)]

        hs = {}
        st = {}

        def pQ(b, t, c0, c1, dl):
            if dl or b not in hs:
                hs[b] = ha_v[S + b * TM:S + (b + 1) * TM, :]
            lhs_ = hs[b]
            pig = plan == 3 and b == 0 and t == 0
            if pig:
                lhs_ = jnp.concatenate([sa_v[...], lhs_], axis=0)
            r = dot_mods(lhs_, lambda lo, hi: wqkv_p[0:D, lo:hi], t * D + 128 * c0, 128 * (c1 - c0), MODS.get(('q', b, t)))
            if pig:
                bias_v[:, 128 * c0:128 * c1] = r[0:8, :]
                bq = r[0:8, :]
                r = r[16:, :]
            elif plan == 3 and b == 1 and t == 0:
                bq = bias_v[:, 128 * c0:128 * c1]
            qk = qkb[b]
            for c in range(c0, c1):
                rc = r[:, 128 * (c - c0):128 * (c - c0 + 1)]
                if t == 0:
                    if plan == 3 and b < 2:
                        rc = _add8(rc, bq[:, 128 * (c - c0):128 * (c - c0 + 1)])
                    qk[QB + c * TM:QB + (c + 1) * TM, :] = rc * (DH ** -0.5 * LOG2E)
                elif t == 1:
                    qk[c * KR + HALO:(c + 1) * KR, :] = rc
                    if b + 1 < NB:
                        qkb[b + 1][c * KR:c * KR + HALO, :] = rc[TM - HALO:TM, :]
                else:
                    vb[b][c * KR + HALO:(c + 1) * KR, :] = rc
                    if b + 1 < NB:
                        vb[b + 1][c * KR:c * KR + HALO, :] = rc[TM - HALO:TM, :]
            return r

        def pW(b):
            a = jnp.dot(ha_v[b * TM:(b + 1) * TM, :], wo_p[0:D, :], preferred_element_type=f32)
            x1b[b][0:TM, :] = xb[b][0:TM, :].astype(f32) + _mul8(a, modv(2))
            return a

        def p1(b, j):
            if b not in st:
                st[b] = dict(y=ha_v[2 * S + b * TM:2 * S + (b + 1) * TM, :], g={}, z=None, n=0)
            lo, hi = FCH[j]
            if b == 0 and j == 0:
                b1_f[...] = jnp.broadcast_to(b1_v[...].astype(f32).reshape(1, F), (8, F))
            w1get = (lambda l_, h_: _upk(w1_p[0:D // 2, l_:h_])) if (rp and b > 0) else (lambda l_, h_: w1_v[0:D, l_:h_])
            u = _add8(dot_mods(st[b]['y'], w1get, lo, hi - lo, MODS.get(('m1', b, j))), b1_f[:, lo:hi])
            t = jnp.tanh(u * (GC0 + GC1 * (u * u)))
            st[b]['g'][j] = (u + u * t).astype(bf16)
            return u

        def epilogue(b, z, c0, c1):
            cs = slice(128 * c0, 128 * c1)
            hg = mod_ref[:, 5 * D + 128 * c0:5 * D + 128 * c1]
            gb2 = mod_ref[:, 6 * D + 128 * c0:6 * D + 128 * c1]
            out_v[b * TM:(b + 1) * TM, cs] = (_add8(x1b[b][0:TM, cs], gb2) + _mul8(z, hg)).astype(bf16)
            ocopy(b, c0, c1)

        def w2get(b, lo, hi, c0, c1):
            if rp and b > 0:
                return _upk(w2_p[lo // 2:hi // 2, c0:c1])
            return w2_v[lo:hi, c0:c1]

        def p2(b, j):
            lo, hi = FCH[j]
            s_ = st[b]
            s_['n'] += 1
            if s_['n'] == 4 and tail and b == NB - 1:
                zs = []
                for c in range(4):
                    zp = jnp.dot(s_['g'][j], w2get(b, lo, hi, 128 * c, 128 * (c + 1)), preferred_element_type=f32)
                    epilogue(b, s_['z'][:, 128 * c:128 * (c + 1)] + zp, c, c + 1)
                    zs.append(zp)
                return jnp.concatenate(zs, axis=1)
            zp = jnp.dot(s_['g'][j], w2get(b, lo, hi, 0, D), preferred_element_type=f32)
            s_['z'] = zp if s_['z'] is None else s_['z'] + zp
            if s_['n'] == 4:
                epilogue(b, s_['z'], 0, 4)
            return zp

        def repack_task(which, k):
            def sA(tokv):
                if which == 1:
                    w1_v[pl.ds(pl.multiple_of(tix[3], 16), 16), 0:128] = tok16(tokv)
                    w1_p[0:D // 2, 128 * k:128 * (k + 1)] = _pk(w1_v[0:D, 128 * k:128 * (k + 1)])
                else:
                    w2_v[pl.ds(pl.multiple_of(tix[5], 16), 16), 0:128] = tok16(tokv)
                    w2_p[64 * k:64 * (k + 1), :] = _pk(w2_v[128 * k:128 * (k + 1), :])
            return [(0, sA)]

        def dur(pc):
            k = pc[0]
            if k == 'q':
                return (pc[4] - pc[3]) * TM
            if k == 'w':
                return 4 * TM
            if k == 'm1' or k == 'm2':
                lo, hi = FCH[pc[2]]
                return (hi - lo) // 128 * TM
            return 0

        fen_last = {}

        def fence(pc, prev_arr):
            k = pc[0]
            if k not in ('q', 'w', 'm1', 'm2') or (k in ('m1', 'm2') and not (rp and pc[1] > 0)):
                return
            key = (pc[1], pc[2]) if k == 'q' else pc[1]
            used = fen_last.setdefault(k, set())
            grp_ = pc[2:] if k != 'w' else 0
            if grp_ in used and prev_arr is not None:
                ref, ti = {'q': (wqkv_p, 6), 'w': (wo_p, 6), 'm1': (w1_p, 6), 'm2': (w2_p, 7)}[k]
                ntl = prev_arr.shape[1] // 128 * NT
                n, r = divmod(int(ntl * fpos / 100), NT)
                ref[pl.ds(pl.multiple_of(tix[ti], 8), 8), 0:128] = pltpu.bitcast(
                    prev_arr[8 * r:8 * r + 8, 128 * n:128 * (n + 1)], u32)
                used.clear()
            used.add(grp_)

        def run_piece(pc, dl):
            k = pc[0]
            if k == 'q':
                return pQ(pc[1], pc[2], pc[3], pc[4], dl)
            if k == 'w':
                return pW(pc[1])
            if k == 'm1':
                return p1(pc[1], pc[2])
            if k == 'm2':
                return p2(pc[1], pc[2])
            if k == 'perm':
                perm_part(pc[1])
            elif k == 'wait':
                wait(*pc[1:])
            elif k == 'mods':
                for n in pc[1:]:
                    mod_tile(n)
            return None

        def run_seq(pieces, groups):
            NP = len(pieces)
            t0s = []
            t = 0
            for pc in pieces:
                t0s.append(t)
                t += dur(pc)
            t0s.append(t)
            sched = {i: [] for i in range(NP)}
            G = 8
            seen = set()
            dlf = []
            for i, pc in enumerate(pieces):
                d = pc[0] in ('wait', 'w')
                if pc[0] in ('q', 'm1'):
                    if (pc[0], pc[1]) not in seen:
                        d = True
                        seen.add((pc[0], pc[1]))
                    elif pc[0] == 'q' and i + 1 < NP and pieces[i + 1][0] == 'wait':
                        d = True
                dlf.append(d)
            live = [i for i in range(NP) if dur(pieces[i]) > 0]
            live_t = [t0s[i] for i in live]
            seq = 0
            for fns, i0, i1, lat in groups:
                lat = lat + max(dt for dt, _ in fns[0])
                dls = [t0s[i] for i in range(i0 + 1, i1 + 1) if dlf[i]] + [t0s[i1 + 1]]
                slots = []
                for i in range(i0, i1 + 1):
                    if i + 1 < NP and pieces[i + 1][0] == 'wait':
                        continue
                    wt = wa if pieces[i][0] == 'm1' else wb
                    for tt in range(t0s[i], t0s[i + 1], G):
                        if any(d - lat <= tt < d for d in dls):
                            continue
                        slots.append((i, tt, wt))
                tot = sum(s_[2] for s_ in slots)
                n = len(fns)
                acc = 0
                kk = 0
                for (i, tt, wt) in slots:
                    while kk < n and kk / n * tot < acc + wt:
                        for dt, fn in fns[kk]:
                            ii = live[bisect.bisect_right(live_t, tt + dt) - 1]
                            sched[ii].append(((tt + dt - t0s[ii]) / dur(pieces[ii]), seq, fn))
                            seq += 1
                        kk += 1
                    acc += wt
                assert kk == n
            prev_arr = None
            for i, pc in enumerate(pieces):
                if fen:
                    fence(pc, prev_arr)
                arr = run_piece(pc, dlf[i])
                prev_arr = arr
                for fr, _, fn in sorted(sched[i], key=lambda t_: (t_[0], t_[1])):
                    ntl = arr.shape[1] // 128 * NT
                    ti = min(int(fr * ntl), ntl - 1)
                    n, r = divmod(ti, NT)
                    fn(arr[8 * r:8 * r + 8, 128 * n:128 * (n + 1)])

        def Qp(b, t, sp=0):
            if sp:
                return [('q', b, t, 0, 4 - sp), ('q', b, t, 4 - sp, 4)]
            return [('q', b, t, 0, 4)]

        def Qs(b, sp=0):
            return Qp(b, 0) + Qp(b, 1) + Qp(b, 2, sp)

        def Wp(b):
            return [('w', b)]

        def Ms(b):
            o = [3, 0, 1, 2] if (tail and b == NB - 1) else [0, 1, 2, 3]
            return [('m1', b, o[0]), ('m1', b, o[1]), ('m2', b, o[0]), ('m1', b, o[2]), ('m2', b, o[1]),
                    ('m1', b, o[3]), ('m2', b, o[2]), ('m2', b, o[3])]

        for c in range(4):
            qkb[0][c * KR:c * KR + HALO, :] = jnp.zeros((HALO, 128), f32)
            vb[0][c * KR:c * KR + HALO, :] = jnp.zeros((HALO, 128), f32)
        cp_tix.wait()
        for i in range(len(TIXV)):
            tix[i] = tix2[0, i]
        if plan == 3:
            wait('c', 'x0', 'wca')
            with SC('ln1_0'):
                silu_init()
                for n in range(4, 8):
                    mod_tile(n)
                for tk in ln1_fns(0):
                    for _, f_ in tk:
                        f_(None)
        else:
            wait('c', 'x0', 'wma', 'x1')
            with SC('ln1_01'):
                silu_init()
                for n in range(8):
                    mod_tile(n)
                for tk in ln1_fns(0) + ln1_fns(1):
                    for _, f_ in tk:
                        f_(None)
        pieces = []
        groups = []
        ix = {}

        def addn(*pcs):
            for pc in pcs:
                ix[pc] = len(pieces)
                pieces.append(pc)

        def grp(fns, a, b_, lat):
            groups.append((fns, ix[a[0]], ix[b_[-1]], lat))

        sp = split
        MODS[('m1', 0, 0)] = [[20], [21], [22], [23]]
        if plan != 3:
            addn(('wait', 'wq'), ('perm', 0), *Qp(0, 0), *Qp(1, 0))
        if plan == 3:
            if bm == 0:
                MODS[('q', 0, 0)] = [[('b', 4), ('b', 8)], [('b', 5), ('b', 9)], [('b', 6), ('b', 10)], [('b', 7), ('b', 11)]]
            else:
                MODS[('q', 0, 0)] = [[('b', 8)], [('b', 9)], [('b', 10)], [('b', 11)]]
            addn(('wait', 'wk'), ('perm', 1), *Qp(0, 1))
            addn(('wait', 'wv', 'x1'), ('perm', 2), *Qp(0, 2), *Qp(1, 1), *Qp(1, 2))
            if r2e == 0:
                MODS[('q', 2, 2)] = [[8], [9], [10], [11]]
                MODS[('q', 3, 0)] = [[12], [13], [14], [15]]
                MODS[('q', 3, 1)] = [[16], [17], [18], [19]]
                addn(('wait', 'wsa', 'wq', 'x2'), ('mods', 0, 1, 2, 3), ('perm', 0), *([('mods', ('b', 4), ('b', 5), ('b', 6), ('b', 7))] if bm else []), *Qp(0, 0), *Qp(1, 0), *Qp(2, 0), *Qp(2, 1, sp))
                addn(('wait', 'x3', 'wo', 'wga', 'wsc', 'x4', 'x5'), *Qp(2, 2), *Qp(3, 0), *Qp(3, 1), *Wp(0), *Qp(3, 2), *Qs(4), *Wp(1), *Qs(5, sp))
                grp(ln1_fns(3), Qp(2, 2), Qp(2, 2), L1h)
            grp(ln1_fns(1), Qp(0, 2), Qp(0, 2), L1h)
            grp(ln1_fns(2), Qp(0, 0), Qp(1, 0), L1)
            grp([t_ for pr_ in zip(fix_fns(1), fix_fns(2)) for t_ in pr_], Qp(1, 0), Qp(1, 0), 100)
            grp(attn_fns(0, mh0), Qp(2, 0), Qp(3, 1), LAh)
            grp(permwo_fns(), Qp(3, 0), Qp(3, 1), LP)
            grp(ln1_fns(4), Qp(3, 0), Qp(3, 2), L1)
            grp(attn_fns(1, mh1), Wp(0), Qs(4), LAh)
            grp(ln23_fns(0), Qp(3, 2), Qs(5, sp), L23)
            grp(ln1_fns(5), Qs(4), Wp(1), L1)
        elif plan == 0:
            MODS[('q', 2, 2)] = [[8, 9, 10], [11, 12, 13], [14, 15, 16], [17, 18, 19]]
            addn(('wait', 'wk', 'wv', 'x2'), ('perm', 1), *Qp(0, 1), ('perm', 2), *Qp(0, 2), *Qp(1, 1), *Qp(1, 2),
                 *Qp(2, 0), *Qp(2, 1, sp))
            addn(('wait', 'wo', 'wga', 'wsc', 'x3', 'x4', 'x5'), *Qp(2, 2), *Wp(0), *Qs(3), *Qs(4), *Wp(1), *Qs(5, sp))
            grp(ln1_fns(2), Qp(0, 1), Qp(1, 2), L1)
            grp(attn_fns(0, mh0), Qp(1, 1), Qp(2, 1, sp), LAh)
            grp(permwo_fns(), Qp(2, 2), Qp(2, 2), LP)
            grp(ln1_fns(3), Qp(2, 2), Wp(0), L1)
            grp(ln23_fns(0), Qs(3), Qs(4), L23)
            grp(ln1_fns(4), Qs(3), Qs(3), L1)
            grp(attn_fns(1, mh1), Wp(0), Qs(4), LAh)
            grp(ln1_fns(5), Qs(4), Wp(1), L1)
        elif plan == 2:
            MODS[('q', 2, 2)] = [[8], [9], [10], [11]]
            MODS[('q', 3, 0)] = [[12], [13], [14], [15]]
            MODS[('q', 3, 1)] = [[16], [17], [18], [19]]
            addn(('wait', 'wk', 'wv', 'x2'), ('perm', 1), *Qp(0, 1), ('perm', 2), *Qp(0, 2), *Qp(1, 1), *Qp(1, 2),
                 *Qp(2, 0), *Qp(2, 1, sp))
            addn(('wait', 'wo', 'wga', 'wsc', 'x3', 'x4', 'x5'), *Qp(2, 2), *Qp(3, 0), *Qp(3, 1), *Wp(0), *Qp(3, 2), *Qs(4), *Wp(1), *Qs(5, sp))
            grp(ln1_fns(2), Qp(0, 1), Qp(1, 2), L1)
            grp(attn_fns(0, mh0), Qp(1, 1), Qp(3, 1) if a0x else Qp(2, 1, sp), LAh)
            grp(ln1_fns(3), Qp(2, 2), Qp(2, 2), L1h)
            grp(permwo_fns(), Qp(3, 0), Qp(3, 1), LP)
            grp(ln1_fns(4), Qp(3, 0), Qp(3, 2), L1)
            grp(attn_fns(1, mh1), Wp(0) if a0x else Qp(3, 0), Qs(4), LAh)
            grp(ln23_fns(0), Qp(3, 2), Qs(5, sp) if a0x else Qs(4), L23)
            grp(ln1_fns(5), Qs(4), Wp(1), L1)
        else:
            MODS[('q', 2, 1)] = [[8, 9], [10, 11], [12], [13]]
            MODS[('q', 2, 2)] = [[14, 15], [16, 17], [18], [19]]
            addn(('wait', 'wk', 'wv', 'x2'), ('perm', 1), *Qp(0, 1), ('perm', 2), *Qp(0, 2), *Qp(1, 1), *Qp(1, 2),
                 *Qp(2, 0, sp))
            addn(('wait', 'x3', 'wo', 'wga', 'wsc', 'x4', 'x5'), *Qp(2, 1), *Qp(2, 2), *Qs(3), *Wp(0), *Qs(4), *Wp(1), *Qs(5, sp))
            grp(ln1_fns(2), Qp(0, 1), Qp(1, 2), L1)
            grp(attn_fns(0, mh0), Qp(1, 1), Qs(3), LAh)
            grp(ln1_fns(3), Qp(2, 1), Qp(2, 2), L1)
            grp(permwo_fns(), Qs(3), Qs(3), LP)
            grp(ln1_fns(4), Qs(3), Wp(0), L1)
            grp(attn_fns(1, mh1), Wp(0), Qs(4), LAh)
            grp(ln23_fns(0), Qs(4), Qs(5, sp), L23)
            grp(ln1_fns(5), Qs(4), Wp(1), L1)
        addn(('wait', 'b1', 'w1', 'w2', 'wgb', 'b2', 'x6', 'x7'), *Ms(0))
        addn(*Wp(2), *Qs(6), *Ms(1), *Wp(3), *Qs(7), *Ms(2))
        for b in (3, 4, 5, 6):
            addn(*Wp(b + 1), *Ms(b))
        addn(*Ms(7))
        grp(ln23_fns(1), Ms(0) if (plan in (1, 3) or a0x) else Qs(5, sp), Ms(0), L23)
        grp(attn_fns(2), Wp(1), Ms(0), LA)
        grp(ln1_fns(6), Ms(0), Ms(0), L1)
        grp(ln23_fns(2), Qs(6), Qs(6), L23)
        if rp:
            grp([repack_task(1 + (k % 2), k // 2) for k in range(28)], Wp(2), Qs(6), 200)
        grp(attn_fns(3), Ms(1), Ms(1), LA)
        grp(ln1_fns(7), Ms(1), Ms(1), L1)
        grp(ln23_fns(3), Qs(7), Qs(7), L23)
        grp(attn_fns(4), Ms(2), Ms(2), LA)
        for b in (3, 4, 5, 6):
            grp(ln23_fns(b + 1), Ms(b), Ms(b), L23)
            if b + 2 < NB:
                grp(attn_fns(b + 2), Ms(b), Ms(b), LA)
        run_seq(pieces, groups)
        for cpy in ocopies:
            cpy.wait()

    def fn(A_x, A_wqkv, A_wo, B_x, B_w1, B_b1, B_w2, B_b2, c, w_mod):
        anyspec = pl.BlockSpec(memory_space=pl.ANY)
        return pl.pallas_call(
            kernel,
            in_specs=[anyspec] * 9,
            out_specs=anyspec,
            out_shape=jax.ShapeDtypeStruct((1, S, D), bf16),
            scratch_shapes=(
                [(pltpu.VMEM((TM // 2 + 8, D), u32) if xre else pltpu.VMEM((TM + 16, D), bf16)) for _ in range(NB)]
                + [pltpu.VMEM((NROWS, 128), f32) for _ in range(NB)]
                + [pltpu.VMEM((TM + 8, D), f32) for _ in range(NB)]
                + [pltpu.VMEM((4 * KR + 8, 128), f32) for _ in range(NB)]
                + [
                pltpu.VMEM((S, D), bf16),
                pltpu.VMEM((D, 3 * D), bf16),
                pltpu.VMEM((D // 2 + 8, 3 * D), u32),
                pltpu.VMEM((D + 16, D), bf16),
                pltpu.VMEM((4, 32 * PW + 8, 128), f32),
                pltpu.VMEM((D // 2 + 8, D), u32),
                pltpu.VMEM((D + 16, F), bf16),
                pltpu.VMEM((F + 16, D), bf16),
                pltpu.VMEM((D, 6 * D), bf16),
                pltpu.VMEM((F,), bf16),
                pltpu.VMEM((D,), bf16),
                pltpu.VMEM((1, D), bf16),
                pltpu.VMEM((8, 7 * D), f32),
                pltpu.VMEM((3 * S // 2, D), u32),
                pltpu.VMEM((D // 2 + 8, F), u32),
                pltpu.VMEM((F // 2 + 8, D), u32),
                pltpu.VMEM((8, F), f32),
                pltpu.VMEM((16, D), bf16),
                pltpu.VMEM((16, D), bf16),
                pltpu.VMEM((8, 3 * D), f32),
                pltpu.VMEM((8, 128), jnp.int32),
                pltpu.SMEM((8, 128), jnp.int32),
                pltpu.SemaphoreType.DMA((len(names),)),
                pltpu.SemaphoreType.DMA((NB + 3,)),
            ]),
            compiler_params=pltpu.CompilerParams(
                vmem_limit_bytes=100 * 1024 * 1024,
            ),
        )(A_x, A_wqkv, A_wo, B_w1, B_b1, B_w2, B_b2, c, w_mod)
    return fn


_impl = make()


@jax.jit
def pallas_adaLN_cond__sliding_local_dilated__mixer_channel_mlp__prompt_kernel(
    A_x: jax.Array,
    A_wqkv: jax.Array,
    A_wo: jax.Array,
    B_x: jax.Array,
    B_w1: jax.Array,
    B_b1: jax.Array,
    B_w2: jax.Array,
    B_b2: jax.Array,
    c: jax.Array,
    w_mod: jax.Array,
):
    return _impl(A_x, A_wqkv, A_wo, B_x, B_w1, B_b1, B_w2, B_b2, c, w_mod)
```

```python
import bisect
import functools

import jax
import jax.numpy as jnp
from jax import lax
import jax.experimental.pallas as pl
import jax.experimental.pallas.tpu as pltpu

S, D, F = 2048, 512, 1792
H, DH, W, DIL = 32, 16, 8, 2
HALO = 16
LOG2E = 1.4426950408889634
EPS = 1e-5
GC0 = 0.7978845608028654
GC1 = 0.7978845608028654 * 0.044715
f32 = jnp.float32
bf16 = jnp.bfloat16
u32 = jnp.uint32
P = functools.partial


def _ln(x):
    m = jnp.mean(x, axis=-1, keepdims=True)
    xc = x - m
    v = jnp.mean(xc * xc, axis=-1, keepdims=True)
    return xc * jnp.exp2(-0.5 * jnp.log2(v + EPS))


def _mul8(x, r8):
    R, N = x.shape
    return (x.reshape(R // 8, 8, N) * r8.reshape(1, 8, N)).reshape(R, N)


def _add8(x, r8):
    R, N = x.shape
    return (x.reshape(R // 8, 8, N) + r8.reshape(1, 8, N)).reshape(R, N)


def make(RC=8, LC=32, L1C=32, wa=10, wb=25, LA=250, L23=150, sa=16, T=250, sb=28,
         DA=450, LAh=250, LP=500, L1h=50, PW=17, D1a=450, L1a=450, D1h=350, D1s=500, L1=300, L1s=300,
         D23h=650, D23s=800, L23h=150, LAa=250, LF=50):
    TM = 256
    NB = S // TM
    KR = TM + HALO
    QB = 4 * KR
    VT = 4 * KR
    TB = QB + 4 * TM
    NROWS = TB + 8
    NT = TM // 8
    FCH = [(0, 512), (512, 1024), (1024, 1536), (1536, 1792)]
    WGROUPS = [('c', 'x0', 'wca', 'tix'), ('wk',), ('wv', 'x1'), ('wsa', 'wq', 'x2'),
               ('x3', 'wo', 'wga', 'wsc', 'x4', 'x5'), ('b1', 'w1', 'w2', 'wgb', 'b2', 'x6', 'x7')]
    SID = {n: i for i, g_ in enumerate(WGROUPS) for n in g_}
    NSEM = len(WGROUPS) + 1

    def kernel(x_hbm, wqkv_hbm, wo_hbm, w1_hbm, b1_hbm, w2_hbm, b2_hbm, c_hbm, wmod_hbm, out_hbm, *scr):
        scr = list(scr)
        xb = [scr.pop(0) for _ in range(NB)]
        qkb = [scr.pop(0) for _ in range(NB)]
        x1b = [scr.pop(0) for _ in range(NB)]
        vb = [scr.pop(0) for _ in range(NB)]
        (out_v, wqkv_v, wqkv_p, wo_v, wo_f, wo_p, w1_v, w2_v, wmod_v, b1_v, b2_v, c_v,
         mod_ref, ha_v, b1_f, sc_v, sa_v, bias_v, qm_v, tix_v, tix2, sems) = scr

        wqkv_p = wqkv_p.bitcast(bf16)
        wo_p = wo_p.bitcast(bf16)
        ha_v = ha_v.bitcast(bf16)
        w1_v = w1_v.bitcast(bf16)
        w2_v = w2_v.bitcast(bf16)

        ocopies = []

        def ocopy(b, c0, c1):
            cpy = pltpu.make_async_copy(out_v.at[pl.ds(b * TM, TM), pl.ds(128 * c0, 128 * (c1 - c0))],
                                        out_hbm.at[0, pl.ds(b * TM, TM), pl.ds(128 * c0, 128 * (c1 - c0))],
                                        sems.at[NSEM - 1])
            ocopies.append(cpy)
            cpy.start()

        def mk(name, src, dst):
            return pltpu.make_async_copy(src, dst, sems.at[SID[name]])

        def wm(lo, hi, name):
            return mk(name, wmod_hbm.at[:, lo * D:hi * D], wmod_v.at[:, lo * D:hi * D])

        cp = dict(
            c=mk('c', c_hbm, c_v),
            wq=mk('wq', wqkv_hbm.at[:, 0:D], wqkv_v.at[:, 0:D]),
            wk=mk('wk', wqkv_hbm.at[:, D:2 * D], wqkv_v.at[:, D:2 * D]),
            wv=mk('wv', wqkv_hbm.at[:, 2 * D:3 * D], wqkv_v.at[:, 2 * D:3 * D]),
            wsa=wm(0, 1, 'wsa'), wca=wm(1, 2, 'wca'), wga=wm(2, 3, 'wga'), wsc=wm(3, 5, 'wsc'), wgb=wm(5, 6, 'wgb'),
            wo=mk('wo', wo_hbm, wo_v.at[pl.ds(0, D), :]),
            w1=mk('w1', w1_hbm, w1_v), w2=mk('w2', w2_hbm, w2_v),
            b1=mk('b1', b1_hbm, b1_v), b2=mk('b2', b2_hbm, b2_v),
            tix=mk('tix', tix_v, tix2),
        )
        for b in range(NB):
            cp['x%d' % b] = mk('x%d' % b, x_hbm.at[0, pl.ds(b * TM, TM), :], xb[b].at[pl.ds(0, TM), :])
        for g_ in WGROUPS:
            for o in g_:
                if o != 'tix':
                    cp[o].start()

        def wait(gi):
            for n in WGROUPS[gi]:
                cp[n].wait()

        TIXV = [TB, TM, 0, D, VT, 8]
        lane0 = lax.broadcasted_iota(jnp.int32, (8, 128), 1)
        tv = jnp.zeros((8, 128), jnp.int32)
        for i, v_ in enumerate(TIXV):
            tv = jnp.where(lane0 == i, v_, tv)
        tix_v[...] = tv
        cp['tix'].start()
        tix = [None] * len(TIXV)

        def silu_init():
            c = c_v[...].astype(f32)
            sc = c * jax.nn.sigmoid(c)
            sc_v[...] = jnp.broadcast_to(sc, (16, D)).astype(bf16)

        def mod_tile(n):
            if isinstance(n, tuple):
                nn = n[1]
                bias_v[0:8, 128 * nn:128 * (nn + 1)] = jnp.dot(sa_v[0:8, :], wqkv_p[:, 128 * nn:128 * (nn + 1)],
                                                               preferred_element_type=f32)
                return
            cs = slice(128 * n, 128 * (n + 1))
            m = jnp.dot(sc_v[0:8, :], wmod_v[:, cs], preferred_element_type=f32)
            if 4 <= n < 8 or 16 <= n < 20:
                m = 1.0 + m
            if n < 4:
                sa_v[:, cs] = jnp.concatenate([m, m], axis=0).astype(bf16)
            if n >= 20:
                b2 = b2_v[...].astype(f32).reshape(1, D)[:, 128 * (n - 20):128 * (n - 19)]
                mod_ref[:, 128 * (n + 4):128 * (n + 5)] = m * b2
                m = 0.5 * m
            mod_ref[:, cs] = m

        def modv(i):
            return mod_ref[:, i * D:(i + 1) * D]

        def perm_init():
            r = lax.broadcasted_iota(jnp.int32, (128, 128), 0)
            cc = lax.broadcasted_iota(jnp.int32, (128, 128), 1)
            for cpi in range(4):
                tgt = ((r & 3) << 5) | (((cpi ^ ((r >> 2) & 3))) << 3) | (r >> 4)
                qm_v[cpi] = jnp.where(cc == tgt, 1.0, 0.0).astype(bf16)

        def perm_part(t):
            lane = lax.broadcasted_iota(jnp.int32, (D // 2, 128), 1)
            e0 = (lane & 4) != 0
            e1 = (lane & 8) != 0
            ch = [pltpu.bitcast(wqkv_v[:, t * D + 128 * c:t * D + 128 * (c + 1)], u32) for c in range(4)]
            res = None
            for cpi in range(4):
                lo_ = jnp.where(e0, ch[cpi ^ 1], ch[cpi ^ 0])
                hi_ = jnp.where(e0, ch[cpi ^ 3], ch[cpi ^ 2])
                mg = pltpu.bitcast(jnp.where(e1, hi_, lo_), bf16)
                rr = jnp.dot(mg, qm_v[cpi], preferred_element_type=f32)
                if cpi == 0:
                    res = rr
                wqkv_p[:, t * D + 128 * cpi:t * D + 128 * (cpi + 1)] = rr.astype(bf16)
            return jnp.concatenate([res[0:TM, :], res[TM:2 * TM, :]], axis=1)

        def dynrows(r, n):
            return pl.ds(pl.multiple_of(tix[2] + r, 16), n)

        def tok16(tokv):
            return jnp.concatenate([tokv, tokv], axis=0).astype(bf16)

        def permwo_task(n):
            def sA(tokv):
                wo_v[pl.ds(pl.multiple_of(tix[3], 16), 16), 0:128] = tok16(tokv)
                wf = wo_v[0:D, 128 * n:128 * (n + 1)].astype(f32)
                for hh in range(H):
                    wo_f[n, pl.ds(hh * PW, 16), :] = wf[16 * hh:16 * hh + 16, :]
                for cpi in range(4):
                    for t in range(4):
                        parts = []
                        for g in range(4):
                            d = ((cpi ^ g) << 2) | t
                            parts.append(wo_f[n, pl.ds(g * 8 * PW + d, 8, stride=PW), :])
                        wo_p[cpi * 128 + t * 32:cpi * 128 + t * 32 + 32, 128 * n:128 * (n + 1)] = (
                            jnp.concatenate(parts, axis=0).astype(bf16))
            return [(0, sA)]

        def ln1_task(b, j):
            r0 = j * L1C
            stt = {}

            def sA(tokv):
                if tokv is not None:
                    xb[b][pl.ds(pl.multiple_of(tix[1], 16), 16), 0:128] = tok16(tokv)
                x = xb[b][r0:r0 + L1C, :].astype(f32)
                hh = _mul8(_ln(x), modv(1))
                if b >= 2:
                    hh = _add8(hh, modv(0))
                stt['h'] = hh.astype(bf16)

            def sB(tokv):
                ha_v[dynrows(S + b * TM + r0, L1C), :] = stt['h']

            return [(0, sA), (D1a if b == 2 else (D1h if b < 6 else D1s), sB)]

        def ln23_task(b, j):
            r0 = j * LC
            stt = {}

            def sA(tokv):
                x1b[b][pl.ds(pl.multiple_of(tix[1], 8), 8), 0:128] = tokv
                h2 = _add8(_mul8(_ln(x1b[b][r0:r0 + LC, :]), modv(4)), modv(3))
                stt['y'] = _ln(h2).astype(bf16)

            def sB(tokv):
                ha_v[dynrows(2 * S + b * TM + r0, LC), :] = stt['y']

            return [(0, sA), (D23h if b == 0 else D23s, sB)]

        attprev = {}

        def attn_task(b, j, micro):
            r0 = j * RC
            qk = qkb[b]
            stt = dict(logits=[], outs=[])

            def qk_step(w, tokv):
                if tokv is not None:
                    qk[pl.ds(pl.multiple_of(tix[0], 8), 8), :] = tokv
                if w == 0:
                    stt['q'] = [qk[QB + c * TM + r0:QB + c * TM + r0 + RC, :] for c in range(4)]
                q = stt['q']
                off = HALO + r0 - DIL * w
                ps_ = [q[c] * qk[pl.ds(c * KR + off, RC), :] for c in range(4)]
                acc = (ps_[0] + ps_[1]) + (ps_[2] + ps_[3])
                if micro:
                    acc = (acc + pltpu.roll(acc, 64, 1)) + (pltpu.roll(acc, 32, 1) + pltpu.roll(acc, 96, 1))
                else:
                    acc = acc + pltpu.roll(acc, 64, 1)
                    acc = acc + pltpu.roll(acc, 32, 1)
                if b == 0 and r0 < DIL * w:
                    row = r0 + lax.broadcasted_iota(jnp.int32, (RC, 128), 0)
                    acc = jnp.where(row >= DIL * w, acc, -1e9 * LOG2E)
                stt['logits'].append(acc)
                if w == W - 1:
                    lg = stt['logits']
                    m = jnp.maximum(jnp.maximum(jnp.maximum(lg[0], lg[1]), jnp.maximum(lg[2], lg[3])),
                                    jnp.maximum(jnp.maximum(lg[4], lg[5]), jnp.maximum(lg[6], lg[7])))
                    ps = [jnp.exp2(l - m) for l in lg]
                    den = ((ps[0] + ps[1]) + (ps[2] + ps[3])) + ((ps[4] + ps[5]) + (ps[6] + ps[7]))
                    r_ = pl.reciprocal(den, approx=True)
                    stt['inv'] = r_ * (2.0 - den * r_)
                    stt['ps'] = ps

            def pv_step(c, tokv):
                if tokv is not None:
                    vb[b][pl.ds(pl.multiple_of(tix[4], 8), 8), :] = tokv
                ps = stt['ps']
                ts = [ps[w] * vb[b][pl.ds(c * KR + HALO + r0 - DIL * w, RC), :] for w in range(W)]
                acc = ((ts[0] + ts[1]) + (ts[2] + ts[3])) + ((ts[4] + ts[5]) + (ts[6] + ts[7]))
                stt['outs'].append(acc * stt['inv'])
                if c == 3:
                    o = jnp.concatenate(stt['outs'], axis=1)
                    if j % 2 == 0:
                        attprev[b] = o
                    else:
                        oo = jnp.concatenate([attprev[b], o], axis=0).astype(bf16)
                        ha_v[dynrows(b * TM + r0 - RC, 2 * RC), :] = oo

            if micro:
                return [(sa * w, P(qk_step, w)) for w in range(W)] + [(T + sb * c, P(pv_step, c)) for c in range(4)]

            def allA(tokv):
                qk_step(0, tokv)
                for w in range(1, W):
                    qk_step(w, None)
                for c in range(3):
                    pv_step(c, None)

            def allB(tokv):
                pv_step(3, None)
            return [(0, allA), (DA, allB)]

        def fix_task(t, b, c):
            def sA(tokv):
                ref = qkb[b] if t == 1 else vb[b]
                bias_v[pl.ds(pl.multiple_of(tix[5], 8), 8), 0:128] = tokv
                lo = c * KR + (HALO if b == 0 else 0)
                hi = c * KR + (HALO if b == 2 else KR)
                ref[lo:hi, :] = _add8(ref[lo:hi, :], bias_v[0:8, t * D + 128 * c:t * D + 128 * (c + 1)])
            return [(0, sA)]

        def attn_fns(b, mi=1):
            return [attn_task(b, j, mi) for j in range(TM // RC)]

        def ln1_fns(b):
            return [ln1_task(b, j) for j in range(TM // L1C)]

        def ln23_fns(b):
            return [ln23_task(b, j) for j in range(TM // LC)]

        hs = {}
        st = {}
        MODS = {}

        def dot_mods(lhs_, wref, c0, ncol, mods):
            if not mods:
                return jnp.dot(lhs_, wref[:, c0:c0 + ncol], preferred_element_type=f32)
            outs = []
            for c in range(ncol // 128):
                outs.append(jnp.dot(lhs_, wref[:, c0 + 128 * c:c0 + 128 * (c + 1)], preferred_element_type=f32))
                for n in mods[c]:
                    mod_tile(n)
            return jnp.concatenate(outs, axis=1)

        def pQ(b, t, c0, c1, dl):
            if dl or b not in hs:
                hs[b] = ha_v[S + b * TM:S + (b + 1) * TM, :]
            lhs_ = hs[b]
            pig = b == 0 and t == 0
            if pig:
                lhs_ = jnp.concatenate([sa_v[...], lhs_], axis=0)
            mods = MODS.get(('q', b, t))
            r = dot_mods(lhs_, wqkv_p, t * D + 128 * c0, 128 * (c1 - c0), mods[c0:c1] if mods else None)
            if pig:
                bq = r[0:8, :]
                bias_v[0:8, 128 * c0:128 * c1] = bq
                r = r[16:, :]
            elif b == 1 and t == 0:
                bq = bias_v[0:8, 128 * c0:128 * c1]
            for c in range(c0, c1):
                rc = r[:, 128 * (c - c0):128 * (c - c0 + 1)]
                if t == 0:
                    if b < 2:
                        rc = _add8(rc, bq[:, 128 * (c - c0):128 * (c - c0 + 1)])
                    qkb[b][QB + c * TM:QB + (c + 1) * TM, :] = rc * (DH ** -0.5 * LOG2E)
                else:
                    bufs = qkb if t == 1 else vb
                    bufs[b][c * KR + HALO:(c + 1) * KR, :] = rc
                    if b + 1 < NB:
                        bufs[b + 1][c * KR:c * KR + HALO, :] = rc[TM - HALO:TM, :]
            return r

        def pW(b):
            a = jnp.dot(ha_v[b * TM:(b + 1) * TM, :], wo_p[...], preferred_element_type=f32)
            x1b[b][0:TM, :] = xb[b][0:TM, :].astype(f32) + _mul8(a, modv(2))
            return a

        def p1(b, j):
            if b not in st:
                st[b] = dict(y=ha_v[2 * S + b * TM:2 * S + (b + 1) * TM, :], g={}, z=None, n=0)
            lo, hi = FCH[j]
            if b == 0 and j == 0:
                b1_f[...] = jnp.broadcast_to(b1_v[...].astype(f32).reshape(1, F), (8, F))
            u = _add8(dot_mods(st[b]['y'], w1_v, lo, hi - lo, MODS.get(('m1', b, j))), b1_f[:, lo:hi])
            t = jnp.tanh(u * (GC0 + GC1 * (u * u)))
            st[b]['g'][j] = (u + u * t).astype(bf16)
            return u

        def epilogue(b, z, c0, c1):
            cs = slice(128 * c0, 128 * c1)
            hg = mod_ref[:, 5 * D + 128 * c0:5 * D + 128 * c1]
            gb2 = mod_ref[:, 6 * D + 128 * c0:6 * D + 128 * c1]
            out_v[b * TM:(b + 1) * TM, cs] = (_add8(x1b[b][0:TM, cs], gb2) + _mul8(z, hg)).astype(bf16)
            ocopy(b, c0, c1)

        def p2(b, j):
            lo, hi = FCH[j]
            s_ = st[b]
            s_['n'] += 1
            if s_['n'] == 4 and b == NB - 1:
                zs = []
                for c in range(4):
                    zp = jnp.dot(s_['g'][j], w2_v[lo:hi, 128 * c:128 * (c + 1)], preferred_element_type=f32)
                    epilogue(b, s_['z'][:, 128 * c:128 * (c + 1)] + zp, c, c + 1)
                    zs.append(zp)
                return jnp.concatenate(zs, axis=1)
            zp = jnp.dot(s_['g'][j], w2_v[lo:hi, :], preferred_element_type=f32)
            s_['z'] = zp if s_['z'] is None else s_['z'] + zp
            if s_['n'] == 4:
                epilogue(b, s_['z'], 0, 4)
            return zp

        def dur(pc):
            k = pc[0]
            if k == 'q':
                return (pc[4] - pc[3]) * TM
            if k == 'w':
                return 4 * TM
            if k == 'perm':
                return D
            if k == 'm1' or k == 'm2':
                lo, hi = FCH[pc[2]]
                return (hi - lo) // 128 * TM
            return 0

        def run_piece(pc, dl):
            k = pc[0]
            if k == 'q':
                return pQ(pc[1], pc[2], pc[3], pc[4], dl)
            if k == 'w':
                return pW(pc[1])
            if k == 'm1':
                return p1(pc[1], pc[2])
            if k == 'm2':
                return p2(pc[1], pc[2])
            if k == 'perm':
                return perm_part(pc[1])
            if k == 'wait':
                wait(pc[1])
            elif k == 'mods':
                for n in pc[1:]:
                    mod_tile(n)
            return None

        pieces, groups, ix = [], [], {}

        def add(*pcs):
            for pc in pcs:
                ix[pc] = len(pieces)
                pieces.append(pc)

        def grp(fns, a, b_, lat):
            groups.append((fns, ix[a[0]], ix[b_[-1]], lat))

        def run_all():
            NP = len(pieces)
            t0s = []
            t = 0
            for pc in pieces:
                t0s.append(t)
                t += dur(pc)
            t0s.append(t)
            sched = {i: [] for i in range(NP)}
            seen = set()
            dlf = []
            for i, pc in enumerate(pieces):
                d = pc[0] in ('wait', 'w')
                if pc[0] in ('q', 'm1'):
                    if (pc[0], pc[1]) not in seen:
                        d = True
                        seen.add((pc[0], pc[1]))
                    elif pc[0] == 'q' and i + 1 < NP and pieces[i + 1][0] == 'wait':
                        d = True
                dlf.append(d)
            live = [i for i in range(NP) if dur(pieces[i]) > 0]
            live_t = [t0s[i] for i in live]
            seq = 0
            for fns, i0, i1, lat in groups:
                lat = lat + max(dt for dt, _ in fns[0])
                dls = [t0s[i] for i in range(i0 + 1, i1 + 1) if dlf[i]] + [t0s[i1 + 1]]
                slots = []
                for i in range(i0, i1 + 1):
                    if i + 1 < NP and pieces[i + 1][0] == 'wait':
                        continue
                    wt = wa if pieces[i][0] == 'm1' else wb
                    for tt in range(t0s[i], t0s[i + 1], 8):
                        if any(d - lat <= tt < d for d in dls):
                            continue
                        slots.append((tt, wt))
                tot = sum(s_[1] for s_ in slots)
                n = len(fns)
                acc = 0
                kk = 0
                for (tt, wt) in slots:
                    while kk < n and kk / n * tot < acc + wt:
                        for dt, fn in fns[kk]:
                            ii = live[bisect.bisect_right(live_t, tt + dt) - 1]
                            sched[ii].append(((tt + dt - t0s[ii]) / dur(pieces[ii]), seq, fn))
                            seq += 1
                        kk += 1
                    acc += wt
                assert kk == n
            for i, pc in enumerate(pieces):
                arr = run_piece(pc, dlf[i])
                for fr, _, fn in sorted(sched[i], key=lambda t_: (t_[0], t_[1])):
                    ntl = arr.shape[1] // 128 * NT
                    ti = min(int(fr * ntl), ntl - 1)
                    n, r = divmod(ti, NT)
                    fn(arr[8 * r:8 * r + 8, 128 * n:128 * (n + 1)])

        def Qp(b, t, sp=0):
            if sp:
                return [('q', b, t, 0, 4 - sp), ('q', b, t, 4 - sp, 4)]
            return [('q', b, t, 0, 4)]

        def Qs(b, sp=0):
            return Qp(b, 0) + Qp(b, 1) + Qp(b, 2, sp)

        def Wp(b):
            return [('w', b)]

        def Ms(b):
            o = [3, 0, 1, 2] if b == NB - 1 else [0, 1, 2, 3]
            return [('m1', b, o[0]), ('m1', b, o[1]), ('m2', b, o[0]), ('m1', b, o[2]), ('m2', b, o[1]),
                    ('m1', b, o[3]), ('m2', b, o[2]), ('m2', b, o[3])]

        for c in range(4):
            qkb[0][c * KR:c * KR + HALO, :] = jnp.zeros((HALO, 128), f32)
            vb[0][c * KR:c * KR + HALO, :] = jnp.zeros((HALO, 128), f32)
        perm_init()
        wait(0)
        for i in range(len(TIXV)):
            tix[i] = tix2[0, i]
        silu_init()
        for n in range(4, 8):
            mod_tile(n)
        for tk in ln1_fns(0):
            for _, f_ in tk:
                f_(None)

        MODS[('q', 0, 0)] = [[('b', 8)], [('b', 9)], [('b', 10)], [('b', 11)]]
        MODS[('q', 2, 2)] = [[8], [9], [10], [11]]
        MODS[('q', 3, 0)] = [[12], [13], [14], [15]]
        MODS[('q', 3, 1)] = [[16], [17], [18], [19]]
        MODS[('m1', 0, 0)] = [[20], [21], [22], [23]]
        add(('wait', 1), ('perm', 1), *Qp(0, 1))
        add(('wait', 2), ('perm', 2), *Qp(0, 2), *Qp(1, 1), *Qp(1, 2))
        add(('wait', 3), ('mods', 0, 1, 2, 3), ('perm', 0), ('mods', ('b', 4), ('b', 5), ('b', 6), ('b', 7)),
            *Qp(0, 0), *Qp(1, 0), *Qp(2, 0), *Qp(2, 1, 1))
        add(('wait', 4), *Qp(2, 2), *Qs(3), *Wp(0), *Qs(4), *Qs(5, 1))
        add(('wait', 5), *Ms(0))
        add(*Wp(1), *Qs(6), *Ms(1), *Wp(2), *Qs(7))
        for b in (2, 3, 4, 5, 6):
            add(*Wp(b + 1), *Ms(b))
        add(*Ms(7))
        grp(ln1_fns(1), [('perm', 2)], Qp(0, 2), L1h)
        grp(ln1_fns(2), [('perm', 0)], Qp(1, 0), L1a)
        grp([fix_task(t, b, c) for b in range(3) for c in range(4) for t in (1, 2)], Qp(1, 0), Qp(1, 0), LF)
        grp(attn_fns(0, 0), Qp(2, 0), Qp(3, 2), LAa)
        grp(ln1_fns(3), Qp(2, 2), Qp(2, 2), L1h)
        grp([permwo_task(n) for n in range(4)], Qp(3, 0), Qp(3, 2), LP)
        grp(ln1_fns(4), Qp(3, 0), Qp(3, 2), L1)
        grp(attn_fns(1, 0), Wp(0), Qs(5, 1), LAh)
        grp(ln23_fns(0), Qp(4, 0), Qs(5, 1), L23h)
        grp(ln1_fns(5), Qs(4), Qs(4), L1)
        grp(attn_fns(2), Ms(0), Ms(0), LA)
        grp(ln1_fns(6), Ms(0), Wp(1), L1s)
        grp(ln23_fns(1), Qs(6), Qs(6), L23)
        grp(attn_fns(3), Ms(1), Ms(1), LA)
        grp(ln1_fns(7), Ms(1), Wp(2), L1s)
        grp(ln23_fns(2), Qs(7), Wp(3), L23)
        for b in (2, 3, 4, 5, 6):
            grp(ln23_fns(b + 1), Ms(b), Ms(b), L23)
            if b + 2 < NB:
                grp(attn_fns(b + 2), Ms(b), Ms(b), LA)
        run_all()
        for cpy in ocopies:
            cpy.wait()

    def fn(A_x, A_wqkv, A_wo, B_x, B_w1, B_b1, B_w2, B_b2, c, w_mod):
        anyspec = pl.BlockSpec(memory_space=pl.ANY)
        return pl.pallas_call(
            kernel,
            in_specs=[anyspec] * 9,
            out_specs=anyspec,
            out_shape=jax.ShapeDtypeStruct((1, S, D), bf16),
            scratch_shapes=(
                [pltpu.VMEM((TM + 16, D), bf16) for _ in range(NB)]
                + [pltpu.VMEM((NROWS, 128), f32) for _ in range(NB)]
                + [pltpu.VMEM((TM + 8, D), f32) for _ in range(NB)]
                + [pltpu.VMEM((VT + 8, 128), f32) for _ in range(NB)]
                + [
                    pltpu.VMEM((S, D), bf16),
                    pltpu.VMEM((D, 3 * D), bf16),
                    pltpu.VMEM((D // 2, 3 * D), u32),
                    pltpu.VMEM((D + 16, D), bf16),
                    pltpu.VMEM((4, H * PW + 8, 128), f32),
                    pltpu.VMEM((D // 2, D), u32),
                    pltpu.VMEM((D // 2, F), u32),
                    pltpu.VMEM((F // 2, D), u32),
                    pltpu.VMEM((D, 6 * D), bf16),
                    pltpu.VMEM((F,), bf16),
                    pltpu.VMEM((D,), bf16),
                    pltpu.VMEM((1, D), bf16),
                    pltpu.VMEM((8, 7 * D), f32),
                    pltpu.VMEM((3 * S // 2, D), u32),
                    pltpu.VMEM((8, F), f32),
                    pltpu.VMEM((16, D), bf16),
                    pltpu.VMEM((16, D), bf16),
                    pltpu.VMEM((16, 3 * D), f32),
                    pltpu.VMEM((4, 128, 128), bf16),
                    pltpu.VMEM((8, 128), jnp.int32),
                    pltpu.SMEM((8, 128), jnp.int32),
                    pltpu.SemaphoreType.DMA((NSEM,)),
                ]),
            compiler_params=pltpu.CompilerParams(
                vmem_limit_bytes=100 * 1024 * 1024,
            ),
        )(A_x, A_wqkv, A_wo, B_w1, B_b1, B_w2, B_b2, c, w_mod)
    return fn


_impl = make()


@jax.jit
def pallas_adaLN_cond__sliding_local_dilated__mixer_channel_mlp__prompt_kernel(
    A_x: jax.Array,
    A_wqkv: jax.Array,
    A_wo: jax.Array,
    B_x: jax.Array,
    B_w1: jax.Array,
    B_b1: jax.Array,
    B_w2: jax.Array,
    B_b2: jax.Array,
    c: jax.Array,
    w_mod: jax.Array,
):
    return _impl(A_x, A_wqkv, A_wo, B_x, B_w1, B_b1, B_w2, B_b2, c, w_mod)
```

```python
import bisect
import functools

import jax
import jax.numpy as jnp
from jax import lax
import jax.experimental.pallas as pl
import jax.experimental.pallas.tpu as pltpu

S, D, F = 2048, 512, 1792
H, DH, W, DIL = 32, 16, 8, 2
HALO = 16
LOG2E = 1.4426950408889634
EPS = 1e-5
GC0 = 0.7978845608028654
GC1 = 0.7978845608028654 * 0.044715
f32 = jnp.float32
bf16 = jnp.bfloat16
u32 = jnp.uint32
P = functools.partial


def _ln(x):
    m = jnp.mean(x, axis=-1, keepdims=True)
    xc = x - m
    v = jnp.mean(xc * xc, axis=-1, keepdims=True)
    return xc * jnp.exp2(-0.5 * jnp.log2(v + EPS))


def _mul8(x, r8):
    R, N = x.shape
    return (x.reshape(R // 8, 8, N) * r8.reshape(1, 8, N)).reshape(R, N)


def _add8(x, r8):
    R, N = x.shape
    return (x.reshape(R // 8, 8, N) + r8.reshape(1, 8, N)).reshape(R, N)


def _pk(x):
    return pltpu.bitcast(x, u32)


def _upk(x):
    return pltpu.bitcast(x, bf16)


def make(RC=8, LC=32, L1C=32, wa=10, wb=25, LA=250, L23=150, sa=16, T=250, sb=28,
         DA=450, LAh=250, LP=500, L1h=50, PW=17, D1a=450, L1a=450, D1h=350, D1s=500, L1=300, L1s=300,
         D23h=650, D23s=800, L23h=150, LAa=250, LF=50):
    TM = 256
    NB = S // TM
    KR = TM + HALO
    QB = 4 * KR
    VT = 4 * KR
    TB = QB + 4 * TM
    NROWS = TB + 8
    NT = TM // 8
    FCH = [(0, 512), (512, 1024), (1024, 1536), (1536, 1792)]
    WGROUPS = [('c', 'x0', 'wca', 'tix'), ('wk',), ('wv', 'x1'), ('wsa', 'wq', 'x2'),
               ('x3', 'wo', 'wga', 'wsc', 'x4', 'x5'), ('b1', 'w1', 'w2', 'wgb', 'b2', 'x6', 'x7')]
    SID = {n: i for i, g_ in enumerate(WGROUPS) for n in g_}
    NSEM = len(WGROUPS) + 1

    def kernel(x_hbm, wqkv_hbm, wo_hbm, w1_hbm, b1_hbm, w2_hbm, b2_hbm, c_hbm, wmod_hbm, out_hbm, *scr):
        scr = list(scr)
        xb = [scr.pop(0) for _ in range(NB)]
        qkb = [scr.pop(0) for _ in range(NB)]
        x1b = [scr.pop(0) for _ in range(NB)]
        vb = [scr.pop(0) for _ in range(NB)]
        (out_v, wqkv_v, wqkv_p, wo_v, wo_f, wo_p, w1_v, w2_v, wmod_v, b1_v, b2_v, c_v,
         mod_ref, ha_v, b1_f, sc_v, sa_v, bias_v, qm_v, tix_v, tix2, sems) = scr

        ocopies = []

        def ocopy(b, c0, c1):
            cpy = pltpu.make_async_copy(out_v.at[pl.ds(b * TM, TM), pl.ds(128 * c0, 128 * (c1 - c0))],
                                        out_hbm.at[0, pl.ds(b * TM, TM), pl.ds(128 * c0, 128 * (c1 - c0))],
                                        sems.at[NSEM - 1])
            ocopies.append(cpy)
            cpy.start()

        def mk(name, src, dst):
            return pltpu.make_async_copy(src, dst, sems.at[SID[name]])

        def wm(lo, hi, name):
            return mk(name, wmod_hbm.at[:, lo * D:hi * D], wmod_v.at[:, lo * D:hi * D])

        cp = dict(
            c=mk('c', c_hbm, c_v),
            wq=mk('wq', wqkv_hbm.at[:, 0:D], wqkv_v.at[:, 0:D]),
            wk=mk('wk', wqkv_hbm.at[:, D:2 * D], wqkv_v.at[:, D:2 * D]),
            wv=mk('wv', wqkv_hbm.at[:, 2 * D:3 * D], wqkv_v.at[:, 2 * D:3 * D]),
            wsa=wm(0, 1, 'wsa'), wca=wm(1, 2, 'wca'), wga=wm(2, 3, 'wga'), wsc=wm(3, 5, 'wsc'), wgb=wm(5, 6, 'wgb'),
            wo=mk('wo', wo_hbm, wo_v.at[pl.ds(0, D), :]),
            w1=mk('w1', w1_hbm, w1_v), w2=mk('w2', w2_hbm, w2_v),
            b1=mk('b1', b1_hbm, b1_v), b2=mk('b2', b2_hbm, b2_v),
            tix=mk('tix', tix_v, tix2),
        )
        for b in range(NB):
            cp['x%d' % b] = mk('x%d' % b, x_hbm.at[0, pl.ds(b * TM, TM), :], xb[b].at[pl.ds(0, TM), :])
        for g_ in WGROUPS:
            for o in g_:
                if o != 'tix':
                    cp[o].start()

        def wait(gi):
            for n in WGROUPS[gi]:
                cp[n].wait()

        TIXV = [TB, TM, 0, D, VT, 8]
        lane0 = lax.broadcasted_iota(jnp.int32, (8, 128), 1)
        tv = jnp.zeros((8, 128), jnp.int32)
        for i, v_ in enumerate(TIXV):
            tv = jnp.where(lane0 == i, v_, tv)
        tix_v[...] = tv
        cp['tix'].start()
        tix = [None] * len(TIXV)

        def silu_init():
            c = c_v[...].astype(f32)
            sc = c * jax.nn.sigmoid(c)
            sc_v[...] = jnp.broadcast_to(sc, (16, D)).astype(bf16)

        def mod_tile(n):
            if isinstance(n, tuple):
                nn = n[1]
                bias_v[0:8, 128 * nn:128 * (nn + 1)] = jnp.dot(sa_v[0:8, :], _upk(wqkv_p[:, 128 * nn:128 * (nn + 1)]),
                                                               preferred_element_type=f32)
                return
            cs = slice(128 * n, 128 * (n + 1))
            m = jnp.dot(sc_v[0:8, :], wmod_v[:, cs], preferred_element_type=f32)
            if 4 <= n < 8 or 16 <= n < 20:
                m = 1.0 + m
            if n < 4:
                sa_v[:, cs] = jnp.concatenate([m, m], axis=0).astype(bf16)
            if n >= 20:
                b2 = b2_v[...].astype(f32).reshape(1, D)[:, 128 * (n - 20):128 * (n - 19)]
                mod_ref[:, 128 * (n + 4):128 * (n + 5)] = m * b2
                m = 0.5 * m
            mod_ref[:, cs] = m

        def modv(i):
            return mod_ref[:, i * D:(i + 1) * D]

        def perm_init():
            r = lax.broadcasted_iota(jnp.int32, (128, 128), 0)
            cc = lax.broadcasted_iota(jnp.int32, (128, 128), 1)
            for cpi in range(4):
                tgt = ((r & 3) << 5) | (((cpi ^ ((r >> 2) & 3))) << 3) | (r >> 4)
                qm_v[cpi] = jnp.where(cc == tgt, 1.0, 0.0).astype(bf16)

        def perm_part(t):
            lane = lax.broadcasted_iota(jnp.int32, (D // 2, 128), 1)
            e0 = (lane & 4) != 0
            e1 = (lane & 8) != 0
            ch = [pltpu.bitcast(wqkv_v[:, t * D + 128 * c:t * D + 128 * (c + 1)], u32) for c in range(4)]
            res = None
            for cpi in range(4):
                lo_ = jnp.where(e0, ch[cpi ^ 1], ch[cpi ^ 0])
                hi_ = jnp.where(e0, ch[cpi ^ 3], ch[cpi ^ 2])
                mg = pltpu.bitcast(jnp.where(e1, hi_, lo_), bf16)
                rr = jnp.dot(mg, qm_v[cpi], preferred_element_type=f32)
                if cpi == 0:
                    res = rr
                wqkv_p[:, t * D + 128 * cpi:t * D + 128 * (cpi + 1)] = _pk(rr.astype(bf16))
            return jnp.concatenate([res[0:TM, :], res[TM:2 * TM, :]], axis=1)

        def dynrows(r, n):
            return pl.ds(pl.multiple_of(tix[2] + r // 2, 8), n // 2)

        def tok16(tokv):
            return jnp.concatenate([tokv, tokv], axis=0).astype(bf16)

        def permwo_task(n):
            def sA(tokv):
                wo_v[pl.ds(pl.multiple_of(tix[3], 16), 16), 0:128] = tok16(tokv)
                wf = wo_v[0:D, 128 * n:128 * (n + 1)].astype(f32)
                for hh in range(H):
                    wo_f[n, pl.ds(hh * PW, 16), :] = wf[16 * hh:16 * hh + 16, :]
                for cpi in range(4):
                    for t in range(4):
                        parts = []
                        for g in range(4):
                            d = ((cpi ^ g) << 2) | t
                            parts.append(wo_f[n, pl.ds(g * 8 * PW + d, 8, stride=PW), :])
                        wo_p[cpi * 64 + t * 16:cpi * 64 + t * 16 + 16, 128 * n:128 * (n + 1)] = _pk(
                            jnp.concatenate(parts, axis=0).astype(bf16))
            return [(0, sA)]

        def ln1_task(b, j):
            r0 = j * L1C
            stt = {}

            def sA(tokv):
                if tokv is not None:
                    xb[b][pl.ds(pl.multiple_of(tix[1], 16), 16), 0:128] = tok16(tokv)
                x = xb[b][r0:r0 + L1C, :].astype(f32)
                hh = _mul8(_ln(x), modv(1))
                if b >= 2:
                    hh = _add8(hh, modv(0))
                stt['h'] = _pk(hh.astype(bf16))

            def sB(tokv):
                ha_v[dynrows(S + b * TM + r0, L1C), :] = stt['h']

            return [(0, sA), (D1a if b == 2 else (D1h if b < 6 else D1s), sB)]

        def ln23_task(b, j):
            r0 = j * LC
            stt = {}

            def sA(tokv):
                x1b[b][pl.ds(pl.multiple_of(tix[1], 8), 8), 0:128] = tokv
                h2 = _add8(_mul8(_ln(x1b[b][r0:r0 + LC, :]), modv(4)), modv(3))
                stt['y'] = _pk(_ln(h2).astype(bf16))

            def sB(tokv):
                ha_v[dynrows(2 * S + b * TM + r0, LC), :] = stt['y']

            return [(0, sA), (D23h if b == 0 else D23s, sB)]

        attprev = {}

        def attn_task(b, j, micro):
            r0 = j * RC
            qk = qkb[b]
            stt = dict(logits=[], outs=[])

            def qk_step(w, tokv):
                if tokv is not None:
                    qk[pl.ds(pl.multiple_of(tix[0], 8), 8), :] = tokv
                if w == 0:
                    stt['q'] = [qk[QB + c * TM + r0:QB + c * TM + r0 + RC, :] for c in range(4)]
                q = stt['q']
                off = HALO + r0 - DIL * w
                ps_ = [q[c] * qk[pl.ds(c * KR + off, RC), :] for c in range(4)]
                acc = (ps_[0] + ps_[1]) + (ps_[2] + ps_[3])
                if micro:
                    acc = (acc + pltpu.roll(acc, 64, 1)) + (pltpu.roll(acc, 32, 1) + pltpu.roll(acc, 96, 1))
                else:
                    acc = acc + pltpu.roll(acc, 64, 1)
                    acc = acc + pltpu.roll(acc, 32, 1)
                if b == 0 and r0 < DIL * w:
                    row = r0 + lax.broadcasted_iota(jnp.int32, (RC, 128), 0)
                    acc = jnp.where(row >= DIL * w, acc, -1e9 * LOG2E)
                stt['logits'].append(acc)
                if w == W - 1:
                    lg = stt['logits']
                    m = jnp.maximum(jnp.maximum(jnp.maximum(lg[0], lg[1]), jnp.maximum(lg[2], lg[3])),
                                    jnp.maximum(jnp.maximum(lg[4], lg[5]), jnp.maximum(lg[6], lg[7])))
                    ps = [jnp.exp2(l - m) for l in lg]
                    den = ((ps[0] + ps[1]) + (ps[2] + ps[3])) + ((ps[4] + ps[5]) + (ps[6] + ps[7]))
                    r_ = pl.reciprocal(den, approx=True)
                    stt['inv'] = r_ * (2.0 - den * r_)
                    stt['ps'] = ps

            def pv_step(c, tokv):
                if tokv is not None:
                    vb[b][pl.ds(pl.multiple_of(tix[4], 8), 8), :] = tokv
                ps = stt['ps']
                ts = [ps[w] * vb[b][pl.ds(c * KR + HALO + r0 - DIL * w, RC), :] for w in range(W)]
                acc = ((ts[0] + ts[1]) + (ts[2] + ts[3])) + ((ts[4] + ts[5]) + (ts[6] + ts[7]))
                stt['outs'].append(acc * stt['inv'])
                if c == 3:
                    o = jnp.concatenate(stt['outs'], axis=1)
                    if j % 2 == 0:
                        attprev[b] = o
                    else:
                        oo = jnp.concatenate([attprev[b], o], axis=0).astype(bf16)
                        ha_v[dynrows(b * TM + r0 - RC, 2 * RC), :] = _pk(oo)

            if micro:
                return [(sa * w, P(qk_step, w)) for w in range(W)] + [(T + sb * c, P(pv_step, c)) for c in range(4)]

            def allA(tokv):
                qk_step(0, tokv)
                for w in range(1, W):
                    qk_step(w, None)
                for c in range(3):
                    pv_step(c, None)

            def allB(tokv):
                pv_step(3, None)
            return [(0, allA), (DA, allB)]

        def fix_task(t, b, c):
            def sA(tokv):
                ref = qkb[b] if t == 1 else vb[b]
                bias_v[pl.ds(pl.multiple_of(tix[5], 8), 8), 0:128] = tokv
                lo = c * KR + (HALO if b == 0 else 0)
                hi = c * KR + (HALO if b == 2 else KR)
                ref[lo:hi, :] = _add8(ref[lo:hi, :], bias_v[0:8, t * D + 128 * c:t * D + 128 * (c + 1)])
            return [(0, sA)]

        def attn_fns(b, mi=1):
            return [attn_task(b, j, mi) for j in range(TM // RC)]

        def ln1_fns(b):
            return [ln1_task(b, j) for j in range(TM // L1C)]

        def ln23_fns(b):
            return [ln23_task(b, j) for j in range(TM // LC)]

        hs = {}
        st = {}
        MODS = {}

        def dot_mods(lhs_, wget, c0, ncol, mods):
            if not mods:
                return jnp.dot(lhs_, wget(c0, c0 + ncol), preferred_element_type=f32)
            outs = []
            for c in range(ncol // 128):
                outs.append(jnp.dot(lhs_, wget(c0 + 128 * c, c0 + 128 * (c + 1)), preferred_element_type=f32))
                for n in mods[c]:
                    mod_tile(n)
            return jnp.concatenate(outs, axis=1)

        def pQ(b, t, c0, c1, dl):
            if dl or b not in hs:
                hs[b] = _upk(ha_v[(S + b * TM) // 2:(S + (b + 1) * TM) // 2, :])
            lhs_ = hs[b]
            pig = b == 0 and t == 0
            if pig:
                lhs_ = jnp.concatenate([sa_v[...], lhs_], axis=0)
            mods = MODS.get(('q', b, t))
            r = dot_mods(lhs_, lambda lo_, hi_: _upk(wqkv_p[:, lo_:hi_]), t * D + 128 * c0, 128 * (c1 - c0), mods[c0:c1] if mods else None)
            if pig:
                bq = r[0:8, :]
                bias_v[0:8, 128 * c0:128 * c1] = bq
                r = r[16:, :]
            elif b == 1 and t == 0:
                bq = bias_v[0:8, 128 * c0:128 * c1]
            for c in range(c0, c1):
                rc = r[:, 128 * (c - c0):128 * (c - c0 + 1)]
                if t == 0:
                    if b < 2:
                        rc = _add8(rc, bq[:, 128 * (c - c0):128 * (c - c0 + 1)])
                    qkb[b][QB + c * TM:QB + (c + 1) * TM, :] = rc * (DH ** -0.5 * LOG2E)
                else:
                    bufs = qkb if t == 1 else vb
                    bufs[b][c * KR + HALO:(c + 1) * KR, :] = rc
                    if b + 1 < NB:
                        bufs[b + 1][c * KR:c * KR + HALO, :] = rc[TM - HALO:TM, :]
            return r

        def pW(b):
            a = jnp.dot(_upk(ha_v[b * TM // 2:(b + 1) * TM // 2, :]), _upk(wo_p[...]), preferred_element_type=f32)
            x1b[b][0:TM, :] = xb[b][0:TM, :].astype(f32) + _mul8(a, modv(2))
            return a

        def p1(b, j):
            if b not in st:
                st[b] = dict(y=_upk(ha_v[(2 * S + b * TM) // 2:(2 * S + (b + 1) * TM) // 2, :]), g={}, z=None, n=0)
            lo, hi = FCH[j]
            if b == 0 and j == 0:
                b1_f[...] = jnp.broadcast_to(b1_v[...].astype(f32).reshape(1, F), (8, F))
            u = _add8(dot_mods(st[b]['y'], lambda lo_, hi_: w1_v[:, lo_:hi_], lo, hi - lo, MODS.get(('m1', b, j))), b1_f[:, lo:hi])
            t = jnp.tanh(u * (GC0 + GC1 * (u * u)))
            st[b]['g'][j] = (u + u * t).astype(bf16)
            return u

        def epilogue(b, z, c0, c1):
            cs = slice(128 * c0, 128 * c1)
            hg = mod_ref[:, 5 * D + 128 * c0:5 * D + 128 * c1]
            gb2 = mod_ref[:, 6 * D + 128 * c0:6 * D + 128 * c1]
            out_v[b * TM:(b + 1) * TM, cs] = (_add8(x1b[b][0:TM, cs], gb2) + _mul8(z, hg)).astype(bf16)
            ocopy(b, c0, c1)

        def p2(b, j):
            lo, hi = FCH[j]
            s_ = st[b]
            s_['n'] += 1
            if s_['n'] == 4 and b == NB - 1:
                zs = []
                for c in range(4):
                    zp = jnp.dot(s_['g'][j], w2_v[lo:hi, 128 * c:128 * (c + 1)], preferred_element_type=f32)
                    epilogue(b, s_['z'][:, 128 * c:128 * (c + 1)] + zp, c, c + 1)
                    zs.append(zp)
                return jnp.concatenate(zs, axis=1)
            zp = jnp.dot(s_['g'][j], w2_v[lo:hi, :], preferred_element_type=f32)
            s_['z'] = zp if s_['z'] is None else s_['z'] + zp
            if s_['n'] == 4:
                epilogue(b, s_['z'], 0, 4)
            return zp

        def dur(pc):
            k = pc[0]
            if k == 'q':
                return (pc[4] - pc[3]) * TM
            if k == 'w':
                return 4 * TM
            if k == 'perm':
                return D
            if k == 'm1' or k == 'm2':
                lo, hi = FCH[pc[2]]
                return (hi - lo) // 128 * TM
            return 0

        def run_piece(pc, dl):
            k = pc[0]
            if k == 'q':
                return pQ(pc[1], pc[2], pc[3], pc[4], dl)
            if k == 'w':
                return pW(pc[1])
            if k == 'm1':
                return p1(pc[1], pc[2])
            if k == 'm2':
                return p2(pc[1], pc[2])
            if k == 'perm':
                return perm_part(pc[1])
            if k == 'wait':
                wait(pc[1])
            elif k == 'mods':
                for n in pc[1:]:
                    mod_tile(n)
            return None

        pieces, groups, ix = [], [], {}

        def add(*pcs):
            for pc in pcs:
                ix[pc] = len(pieces)
                pieces.append(pc)

        def grp(fns, a, b_, lat):
            groups.append((fns, ix[a[0]], ix[b_[-1]], lat))

        def run_all():
            NP = len(pieces)
            t0s = []
            t = 0
            for pc in pieces:
                t0s.append(t)
                t += dur(pc)
            t0s.append(t)
            sched = {i: [] for i in range(NP)}
            seen = set()
            dlf = []
            for i, pc in enumerate(pieces):
                d = pc[0] in ('wait', 'w')
                if pc[0] in ('q', 'm1'):
                    if (pc[0], pc[1]) not in seen:
                        d = True
                        seen.add((pc[0], pc[1]))
                    elif pc[0] == 'q' and i + 1 < NP and pieces[i + 1][0] == 'wait':
                        d = True
                dlf.append(d)
            live = [i for i in range(NP) if dur(pieces[i]) > 0]
            live_t = [t0s[i] for i in live]
            seq = 0
            for fns, i0, i1, lat in groups:
                lat = lat + max(dt for dt, _ in fns[0])
                dls = [t0s[i] for i in range(i0 + 1, i1 + 1) if dlf[i]] + [t0s[i1 + 1]]
                slots = []
                for i in range(i0, i1 + 1):
                    if i + 1 < NP and pieces[i + 1][0] == 'wait':
                        continue
                    wt = wa if pieces[i][0] == 'm1' else wb
                    for tt in range(t0s[i], t0s[i + 1], 8):
                        if any(d - lat <= tt < d for d in dls):
                            continue
                        slots.append((tt, wt))
                tot = sum(s_[1] for s_ in slots)
                n = len(fns)
                acc = 0
                kk = 0
                for (tt, wt) in slots:
                    while kk < n and kk / n * tot < acc + wt:
                        for dt, fn in fns[kk]:
                            ii = live[bisect.bisect_right(live_t, tt + dt) - 1]
                            sched[ii].append(((tt + dt - t0s[ii]) / dur(pieces[ii]), seq, fn))
                            seq += 1
                        kk += 1
                    acc += wt
                assert kk == n
            for i, pc in enumerate(pieces):
                arr = run_piece(pc, dlf[i])
                for fr, _, fn in sorted(sched[i], key=lambda t_: (t_[0], t_[1])):
                    ntl = arr.shape[1] // 128 * NT
                    ti = min(int(fr * ntl), ntl - 1)
                    n, r = divmod(ti, NT)
                    fn(arr[8 * r:8 * r + 8, 128 * n:128 * (n + 1)])

        def Qp(b, t, sp=0):
            if sp:
                return [('q', b, t, 0, 4 - sp), ('q', b, t, 4 - sp, 4)]
            return [('q', b, t, 0, 4)]

        def Qs(b, sp=0):
            return Qp(b, 0) + Qp(b, 1) + Qp(b, 2, sp)

        def Wp(b):
            return [('w', b)]

        def Ms(b):
            o = [3, 0, 1, 2] if b == NB - 1 else [0, 1, 2, 3]
            return [('m1', b, o[0]), ('m1', b, o[1]), ('m2', b, o[0]), ('m1', b, o[2]), ('m2', b, o[1]),
                    ('m1', b, o[3]), ('m2', b, o[2]), ('m2', b, o[3])]

        for c in range(4):
            qkb[0][c * KR:c * KR + HALO, :] = jnp.zeros((HALO, 128), f32)
            vb[0][c * KR:c * KR + HALO, :] = jnp.zeros((HALO, 128), f32)
        perm_init()
        wait(0)
        for i in range(len(TIXV)):
            tix[i] = tix2[0, i]
        silu_init()
        for n in range(4, 8):
            mod_tile(n)
        for tk in ln1_fns(0):
            for _, f_ in tk:
                f_(None)

        MODS[('q', 0, 0)] = [[('b', 8)], [('b', 9)], [('b', 10)], [('b', 11)]]
        MODS[('q', 2, 2)] = [[8], [9], [10], [11]]
        MODS[('q', 3, 0)] = [[12], [13], [14], [15]]
        MODS[('q', 3, 1)] = [[16], [17], [18], [19]]
        MODS[('m1', 0, 0)] = [[20], [21], [22], [23]]
        add(('wait', 1), ('perm', 1), *Qp(0, 1))
        add(('wait', 2), ('perm', 2), *Qp(0, 2), *Qp(1, 1), *Qp(1, 2))
        add(('wait', 3), ('mods', 0, 1, 2, 3), ('perm', 0), ('mods', ('b', 4), ('b', 5), ('b', 6), ('b', 7)),
            *Qp(0, 0), *Qp(1, 0), *Qp(2, 0), *Qp(2, 1, 1))
        add(('wait', 4), *Qp(2, 2), *Qs(3), *Wp(0), *Qs(4), *Qs(5, 1))
        add(('wait', 5), *Ms(0))
        add(*Wp(1), *Qs(6), *Ms(1), *Wp(2), *Qs(7))
        for b in (2, 3, 4, 5, 6):
            add(*Wp(b + 1), *Ms(b))
        add(*Ms(7))
        grp(ln1_fns(1), [('perm', 2)], Qp(0, 2), L1h)
        grp(ln1_fns(2), [('perm', 0)], Qp(1, 0), L1a)
        grp([fix_task(t, b, c) for b in range(3) for c in range(4) for t in (1, 2)], Qp(1, 0), Qp(1, 0), LF)
        grp(attn_fns(0, 0), Qp(2, 0), Qp(3, 2), LAa)
        grp(ln1_fns(3), Qp(2, 2), Qp(2, 2), L1h)
        grp([permwo_task(n) for n in range(4)], Qp(3, 0), Qp(3, 2), LP)
        grp(ln1_fns(4), Qp(3, 0), Qp(3, 2), L1)
        grp(attn_fns(1, 0), Wp(0), Qs(5, 1), LAh)
        grp(ln23_fns(0), Qp(4, 0), Qs(5, 1), L23h)
        grp(ln1_fns(5), Qs(4), Qs(4), L1)
        grp(attn_fns(2), Ms(0), Ms(0), LA)
        grp(ln1_fns(6), Ms(0), Wp(1), L1s)
        grp(ln23_fns(1), Qs(6), Qs(6), L23)
        grp(attn_fns(3), Ms(1), Ms(1), LA)
        grp(ln1_fns(7), Ms(1), Wp(2), L1s)
        grp(ln23_fns(2), Qs(7), Wp(3), L23)
        for b in (2, 3, 4, 5, 6):
            grp(ln23_fns(b + 1), Ms(b), Ms(b), L23)
            if b + 2 < NB:
                grp(attn_fns(b + 2), Ms(b), Ms(b), LA)
        run_all()
        for cpy in ocopies:
            cpy.wait()

    def fn(A_x, A_wqkv, A_wo, B_x, B_w1, B_b1, B_w2, B_b2, c, w_mod):
        anyspec = pl.BlockSpec(memory_space=pl.ANY)
        return pl.pallas_call(
            kernel,
            in_specs=[anyspec] * 9,
            out_specs=anyspec,
            out_shape=jax.ShapeDtypeStruct((1, S, D), bf16),
            scratch_shapes=(
                [pltpu.VMEM((TM + 16, D), bf16) for _ in range(NB)]
                + [pltpu.VMEM((NROWS, 128), f32) for _ in range(NB)]
                + [pltpu.VMEM((TM + 8, D), f32) for _ in range(NB)]
                + [pltpu.VMEM((VT + 8, 128), f32) for _ in range(NB)]
                + [
                    pltpu.VMEM((S, D), bf16),
                    pltpu.VMEM((D, 3 * D), bf16),
                    pltpu.VMEM((D // 2, 3 * D), u32),
                    pltpu.VMEM((D + 16, D), bf16),
                    pltpu.VMEM((4, H * PW + 8, 128), f32),
                    pltpu.VMEM((D // 2, D), u32),
                    pltpu.VMEM((D, F), bf16),
                    pltpu.VMEM((F, D), bf16),
                    pltpu.VMEM((D, 6 * D), bf16),
                    pltpu.VMEM((F,), bf16),
                    pltpu.VMEM((D,), bf16),
                    pltpu.VMEM((1, D), bf16),
                    pltpu.VMEM((8, 7 * D), f32),
                    pltpu.VMEM((3 * S // 2, D), u32),
                    pltpu.VMEM((8, F), f32),
                    pltpu.VMEM((16, D), bf16),
                    pltpu.VMEM((16, D), bf16),
                    pltpu.VMEM((16, 3 * D), f32),
                    pltpu.VMEM((4, 128, 128), bf16),
                    pltpu.VMEM((8, 128), jnp.int32),
                    pltpu.SMEM((8, 128), jnp.int32),
                    pltpu.SemaphoreType.DMA((NSEM,)),
                ]),
            compiler_params=pltpu.CompilerParams(
                vmem_limit_bytes=100 * 1024 * 1024,
            ),
        )(A_x, A_wqkv, A_wo, B_w1, B_b1, B_w2, B_b2, c, w_mod)
    return fn


_impl = make()


@jax.jit
def pallas_adaLN_cond__sliding_local_dilated__mixer_channel_mlp__prompt_kernel(
    A_x: jax.Array,
    A_wqkv: jax.Array,
    A_wo: jax.Array,
    B_x: jax.Array,
    B_w1: jax.Array,
    B_b1: jax.Array,
    B_w2: jax.Array,
    B_b2: jax.Array,
    c: jax.Array,
    w_mod: jax.Array,
):
    return _impl(A_x, A_wqkv, A_wo, B_x, B_w1, B_b1, B_w2, B_b2, c, w_mod)
```

```python
import bisect
import functools

import jax
import jax.numpy as jnp
from jax import lax
import jax.experimental.pallas as pl
import jax.experimental.pallas.tpu as pltpu

S, D, F = 2048, 512, 1792
H, DH, W, DIL = 32, 16, 8, 2
HALO = 16
LOG2E = 1.4426950408889634
EPS = 1e-5
GC0 = 0.7978845608028654
GC1 = 0.7978845608028654 * 0.044715
f32 = jnp.float32
bf16 = jnp.bfloat16
u32 = jnp.uint32
P = functools.partial


def _ln(x):
    m = jnp.mean(x, axis=-1, keepdims=True)
    xc = x - m
    v = jnp.mean(xc * xc, axis=-1, keepdims=True)
    return xc * jnp.exp2(-0.5 * jnp.log2(v + EPS))


def _mul8(x, r8):
    R, N = x.shape
    return (x.reshape(R // 8, 8, N) * r8.reshape(1, 8, N)).reshape(R, N)


def _add8(x, r8):
    R, N = x.shape
    return (x.reshape(R // 8, 8, N) + r8.reshape(1, 8, N)).reshape(R, N)


def _pk(x):
    return pltpu.bitcast(x, u32)


def _upk(x):
    return pltpu.bitcast(x, bf16)


def make(RC=8, LC=32, L1C=32, wa=10, wb=25, LA=250, L23=150, sa=16, T=250, sb=28,
         DA=450, LAh=250, LP=500, L1h=50, PW=17, D1a=450, L1a=450, D1h=350, D1s=500, L1=300, L1s=300,
         D23h=650, D23s=800, L23h=150, LAa=250, LF=50):
    TM = 256
    NB = S // TM
    KR = TM + HALO
    QB = 4 * KR
    VT = 4 * KR
    TB = QB + 4 * TM
    NROWS = TB + 8
    NT = TM // 8
    FCH = [(0, 512), (512, 1024), (1024, 1536), (1536, 1792)]
    WGROUPS = [('c', 'x0', 'wca', 'tix'), ('wk',), ('wv', 'x1'), ('wsa', 'wq', 'x2'),
               ('x3', 'wo', 'wga', 'wsb', 'wcb', 'x4', 'x5'), ('b1', 'w1', 'w2', 'wgb', 'b2', 'x6', 'x7')]
    SID = {n: i for i, g_ in enumerate(WGROUPS) for n in g_}
    NSEM = len(WGROUPS) + 1

    def kernel(x_hbm, wqkv_hbm, wo_hbm, w1_hbm, b1_hbm, w2_hbm, b2_hbm, c_hbm, wmod_hbm, out_hbm, *scr):
        scr = list(scr)
        xb = [scr.pop(0) for _ in range(NB)]
        qkb = [scr.pop(0) for _ in range(NB)]
        x1b = [scr.pop(0) for _ in range(NB)]
        vb = [scr.pop(0) for _ in range(NB)]
        outb = [scr.pop(0) for _ in range(NB - 1)]
        outl = [scr.pop(0) for _ in range(4)]
        wraw = [scr.pop(0) for _ in range(3)]
        wmodb = [scr.pop(0) for _ in range(6)]
        (wqkv_p, wo_v, wo_f, wo_p, w1_v, w2_v, b1_v, b2_v, c_v,
         mod_ref, ha_v, b1_f, sc_v, sa_v, bias_v, qm_v, tix_v, tix2, sems) = scr

        ocopies = []

        def ocopy(src, b, c0, c1):
            cpy = pltpu.make_async_copy(src, out_hbm.at[0, pl.ds(b * TM, TM), pl.ds(128 * c0, 128 * (c1 - c0))],
                                        sems.at[NSEM - 1])
            ocopies.append(cpy)
            cpy.start()

        def mk(name, src, dst):
            return pltpu.make_async_copy(src, dst, sems.at[SID[name]])

        def wm(i, name):
            return mk(name, wmod_hbm.at[:, i * D:(i + 1) * D], wmodb[i])

        cp = dict(
            c=mk('c', c_hbm, c_v),
            wq=mk('wq', wqkv_hbm.at[:, 0:D], wraw[0]),
            wk=mk('wk', wqkv_hbm.at[:, D:2 * D], wraw[1]),
            wv=mk('wv', wqkv_hbm.at[:, 2 * D:3 * D], wraw[2]),
            wsa=wm(0, 'wsa'), wca=wm(1, 'wca'), wga=wm(2, 'wga'), wsb=wm(3, 'wsb'), wcb=wm(4, 'wcb'), wgb=wm(5, 'wgb'),
            wo=mk('wo', wo_hbm, wo_v.at[pl.ds(0, D), :]),
            w1=mk('w1', w1_hbm, w1_v), w2=mk('w2', w2_hbm, w2_v),
            b1=mk('b1', b1_hbm, b1_v), b2=mk('b2', b2_hbm, b2_v),
            tix=mk('tix', tix_v, tix2),
        )
        for b in range(NB):
            cp['x%d' % b] = mk('x%d' % b, x_hbm.at[0, pl.ds(b * TM, TM), :], xb[b].at[pl.ds(0, TM), :])
        for g_ in WGROUPS:
            for o in g_:
                if o != 'tix':
                    cp[o].start()

        def wait(gi):
            for n in WGROUPS[gi]:
                cp[n].wait()

        TIXV = [TB, TM, 0, D, VT, 8]
        lane0 = lax.broadcasted_iota(jnp.int32, (8, 128), 1)
        tv = jnp.zeros((8, 128), jnp.int32)
        for i, v_ in enumerate(TIXV):
            tv = jnp.where(lane0 == i, v_, tv)
        tix_v[...] = tv
        cp['tix'].start()
        tix = [None] * len(TIXV)

        def silu_init():
            c = c_v[...].astype(f32)
            sc = c * jax.nn.sigmoid(c)
            sc_v[...] = jnp.broadcast_to(sc, (16, D)).astype(bf16)

        def mod_tile(n):
            if isinstance(n, tuple):
                nn = n[1]
                bias_v[0:8, 128 * nn:128 * (nn + 1)] = jnp.dot(sa_v[0:8, :], _upk(wqkv_p[:, 128 * nn:128 * (nn + 1)]),
                                                               preferred_element_type=f32)
                return
            cs = slice(128 * n, 128 * (n + 1))
            m = jnp.dot(sc_v[0:8, :], wmodb[n // 4][:, 128 * (n % 4):128 * (n % 4 + 1)], preferred_element_type=f32)
            if 4 <= n < 8 or 16 <= n < 20:
                m = 1.0 + m
            if n < 4:
                sa_v[:, cs] = jnp.concatenate([m, m], axis=0).astype(bf16)
            if n >= 20:
                b2 = b2_v[...].astype(f32).reshape(1, D)[:, 128 * (n - 20):128 * (n - 19)]
                mod_ref[:, 128 * (n + 4):128 * (n + 5)] = m * b2
                m = 0.5 * m
            mod_ref[:, cs] = m

        def modv(i):
            return mod_ref[:, i * D:(i + 1) * D]

        def perm_init():
            r = lax.broadcasted_iota(jnp.int32, (128, 128), 0)
            cc = lax.broadcasted_iota(jnp.int32, (128, 128), 1)
            for cpi in range(4):
                tgt = ((r & 3) << 5) | (((cpi ^ ((r >> 2) & 3))) << 3) | (r >> 4)
                qm_v[cpi] = jnp.where(cc == tgt, 1.0, 0.0).astype(bf16)

        def perm_part(t):
            lane = lax.broadcasted_iota(jnp.int32, (D // 2, 128), 1)
            e0 = (lane & 4) != 0
            e1 = (lane & 8) != 0
            ch = [pltpu.bitcast(wraw[t][:, 128 * c:128 * (c + 1)], u32) for c in range(4)]
            res = None
            for cpi in range(4):
                lo_ = jnp.where(e0, ch[cpi ^ 1], ch[cpi ^ 0])
                hi_ = jnp.where(e0, ch[cpi ^ 3], ch[cpi ^ 2])
                mg = pltpu.bitcast(jnp.where(e1, hi_, lo_), bf16)
                rr = jnp.dot(mg, qm_v[cpi], preferred_element_type=f32)
                if cpi == 0:
                    res = rr
                wqkv_p[:, t * D + 128 * cpi:t * D + 128 * (cpi + 1)] = _pk(rr.astype(bf16))
            return jnp.concatenate([res[0:TM, :], res[TM:2 * TM, :]], axis=1)

        def dynrows(r, n):
            return pl.ds(pl.multiple_of(tix[2] + r // 2, 8), n // 2)

        def tok16(tokv):
            return jnp.concatenate([tokv, tokv], axis=0).astype(bf16)

        def permwo_task(n):
            def sA(tokv):
                wo_v[pl.ds(pl.multiple_of(tix[3], 16), 16), 0:128] = tok16(tokv)
                wf = wo_v[0:D, 128 * n:128 * (n + 1)].astype(f32)
                for hh in range(H):
                    wo_f[n, pl.ds(hh * PW, 16), :] = wf[16 * hh:16 * hh + 16, :]
                for cpi in range(4):
                    for t in range(4):
                        parts = []
                        for g in range(4):
                            d = ((cpi ^ g) << 2) | t
                            parts.append(wo_f[n, pl.ds(g * 8 * PW + d, 8, stride=PW), :])
                        wo_p[cpi * 64 + t * 16:cpi * 64 + t * 16 + 16, 128 * n:128 * (n + 1)] = _pk(
                            jnp.concatenate(parts, axis=0).astype(bf16))
            return [(0, sA)]

        def ln1_task(b, j):
            r0 = j * L1C
            stt = {}

            def sA(tokv):
                if tokv is not None:
                    xb[b][pl.ds(pl.multiple_of(tix[1], 16), 16), 0:128] = tok16(tokv)
                x = xb[b][r0:r0 + L1C, :].astype(f32)
                hh = _mul8(_ln(x), modv(1))
                if b >= 2:
                    hh = _add8(hh, modv(0))
                stt['h'] = _pk(hh.astype(bf16))

            def sB(tokv):
                ha_v[dynrows(S + b * TM + r0, L1C), :] = stt['h']

            return [(0, sA), (D1a if b == 2 else (D1h if b < 6 else D1s), sB)]

        def ln23_task(b, j):
            r0 = j * LC
            stt = {}

            def sA(tokv):
                x1b[b][pl.ds(pl.multiple_of(tix[1], 8), 8), 0:128] = tokv
                h2 = _add8(_mul8(_ln(x1b[b][r0:r0 + LC, :]), modv(4)), modv(3))
                stt['y'] = _pk(_ln(h2).astype(bf16))

            def sB(tokv):
                ha_v[dynrows(2 * S + b * TM + r0, LC), :] = stt['y']

            return [(0, sA), (D23h if b == 0 else D23s, sB)]

        attprev = {}

        def attn_task(b, j, micro):
            r0 = j * RC
            qk = qkb[b]
            stt = dict(logits=[], outs=[])

            def qk_step(w, tokv):
                if tokv is not None:
                    qk[pl.ds(pl.multiple_of(tix[0], 8), 8), :] = tokv
                if w == 0:
                    stt['q'] = [qk[QB + c * TM + r0:QB + c * TM + r0 + RC, :] for c in range(4)]
                q = stt['q']
                off = HALO + r0 - DIL * w
                ps_ = [q[c] * qk[pl.ds(c * KR + off, RC), :] for c in range(4)]
                acc = (ps_[0] + ps_[1]) + (ps_[2] + ps_[3])
                if micro:
                    acc = (acc + pltpu.roll(acc, 64, 1)) + (pltpu.roll(acc, 32, 1) + pltpu.roll(acc, 96, 1))
                else:
                    acc = acc + pltpu.roll(acc, 64, 1)
                    acc = acc + pltpu.roll(acc, 32, 1)
                if b == 0 and r0 < DIL * w:
                    row = r0 + lax.broadcasted_iota(jnp.int32, (RC, 128), 0)
                    acc = jnp.where(row >= DIL * w, acc, -1e9 * LOG2E)
                stt['logits'].append(acc)
                if w == W - 1:
                    lg = stt['logits']
                    m = jnp.maximum(jnp.maximum(jnp.maximum(lg[0], lg[1]), jnp.maximum(lg[2], lg[3])),
                                    jnp.maximum(jnp.maximum(lg[4], lg[5]), jnp.maximum(lg[6], lg[7])))
                    ps = [jnp.exp2(l - m) for l in lg]
                    den = ((ps[0] + ps[1]) + (ps[2] + ps[3])) + ((ps[4] + ps[5]) + (ps[6] + ps[7]))
                    r_ = pl.reciprocal(den, approx=True)
                    stt['inv'] = r_ * (2.0 - den * r_)
                    stt['ps'] = ps

            def pv_step(c, tokv):
                if tokv is not None:
                    vb[b][pl.ds(pl.multiple_of(tix[4], 8), 8), :] = tokv
                ps = stt['ps']
                ts = [ps[w] * vb[b][pl.ds(c * KR + HALO + r0 - DIL * w, RC), :] for w in range(W)]
                acc = ((ts[0] + ts[1]) + (ts[2] + ts[3])) + ((ts[4] + ts[5]) + (ts[6] + ts[7]))
                stt['outs'].append(acc * stt['inv'])
                if c == 3:
                    o = jnp.concatenate(stt['outs'], axis=1)
                    if j % 2 == 0:
                        attprev[b] = o
                    else:
                        oo = jnp.concatenate([attprev[b], o], axis=0).astype(bf16)
                        ha_v[dynrows(b * TM + r0 - RC, 2 * RC), :] = _pk(oo)

            if micro:
                return [(sa * w, P(qk_step, w)) for w in range(W)] + [(T + sb * c, P(pv_step, c)) for c in range(4)]

            def allA(tokv):
                qk_step(0, tokv)
                for w in range(1, W):
                    qk_step(w, None)
                for c in range(3):
                    pv_step(c, None)

            def allB(tokv):
                pv_step(3, None)
            return [(0, allA), (DA, allB)]

        def fix_task(t, b, c):
            def sA(tokv):
                ref = qkb[b] if t == 1 else vb[b]
                bias_v[pl.ds(pl.multiple_of(tix[5], 8), 8), 0:128] = tokv
                lo = c * KR + (HALO if b == 0 else 0)
                hi = c * KR + (HALO if b == 2 else KR)
                ref[lo:hi, :] = _add8(ref[lo:hi, :], bias_v[0:8, t * D + 128 * c:t * D + 128 * (c + 1)])
            return [(0, sA)]

        def attn_fns(b, mi=1):
            return [attn_task(b, j, mi) for j in range(TM // RC)]

        def ln1_fns(b):
            return [ln1_task(b, j) for j in range(TM // L1C)]

        def ln23_fns(b):
            return [ln23_task(b, j) for j in range(TM // LC)]

        hs = {}
        st = {}
        MODS = {}

        def dot_mods(lhs_, wget, c0, ncol, mods):
            if not mods:
                return jnp.dot(lhs_, wget(c0, c0 + ncol), preferred_element_type=f32)
            outs = []
            for c in range(ncol // 128):
                outs.append(jnp.dot(lhs_, wget(c0 + 128 * c, c0 + 128 * (c + 1)), preferred_element_type=f32))
                for n in mods[c]:
                    mod_tile(n)
            return jnp.concatenate(outs, axis=1)

        def pQ(b, t, c0, c1, dl):
            if dl or b not in hs:
                hs[b] = _upk(ha_v[(S + b * TM) // 2:(S + (b + 1) * TM) // 2, :])
            lhs_ = hs[b]
            pig = b == 0 and t == 0
            if pig:
                lhs_ = jnp.concatenate([sa_v[...], lhs_], axis=0)
            mods = MODS.get(('q', b, t))
            r = dot_mods(lhs_, lambda lo_, hi_: _upk(wqkv_p[:, lo_:hi_]), t * D + 128 * c0, 128 * (c1 - c0), mods[c0:c1] if mods else None)
            if pig:
                bq = r[0:8, :]
                bias_v[0:8, 128 * c0:128 * c1] = bq
                r = r[16:, :]
            elif b == 1 and t == 0:
                bq = bias_v[0:8, 128 * c0:128 * c1]
            for c in range(c0, c1):
                rc = r[:, 128 * (c - c0):128 * (c - c0 + 1)]
                if t == 0:
                    if b < 2:
                        rc = _add8(rc, bq[:, 128 * (c - c0):128 * (c - c0 + 1)])
                    qkb[b][QB + c * TM:QB + (c + 1) * TM, :] = rc * (DH ** -0.5 * LOG2E)
                else:
                    bufs = qkb if t == 1 else vb
                    bufs[b][c * KR + HALO:(c + 1) * KR, :] = rc
                    if b + 1 < NB:
                        bufs[b + 1][c * KR:c * KR + HALO, :] = rc[TM - HALO:TM, :]
            return r

        def pW(b):
            a = jnp.dot(_upk(ha_v[b * TM // 2:(b + 1) * TM // 2, :]), _upk(wo_p[...]), preferred_element_type=f32)
            x1b[b][0:TM, :] = xb[b][0:TM, :].astype(f32) + _mul8(a, modv(2))
            return a

        def p1(b, j):
            if b not in st:
                st[b] = dict(y=_upk(ha_v[(2 * S + b * TM) // 2:(2 * S + (b + 1) * TM) // 2, :]), g={}, z=None, n=0)
            lo, hi = FCH[j]
            if b == 0 and j == 0:
                b1_f[...] = jnp.broadcast_to(b1_v[...].astype(f32).reshape(1, F), (8, F))
            u = _add8(dot_mods(st[b]['y'], lambda lo_, hi_: w1_v[:, lo_:hi_], lo, hi - lo, MODS.get(('m1', b, j))), b1_f[:, lo:hi])
            t = jnp.tanh(u * (GC0 + GC1 * (u * u)))
            st[b]['g'][j] = (u + u * t).astype(bf16)
            return u

        def epilogue(b, z, c0, c1):
            cs = slice(128 * c0, 128 * c1)
            hg = mod_ref[:, 5 * D + 128 * c0:5 * D + 128 * c1]
            gb2 = mod_ref[:, 6 * D + 128 * c0:6 * D + 128 * c1]
            dst = outl[c0] if b == NB - 1 else outb[b]
            dst[...] = (_add8(x1b[b][0:TM, cs], gb2) + _mul8(z, hg)).astype(bf16)
            ocopy(dst, b, c0, c1)

        def p2(b, j):
            lo, hi = FCH[j]
            s_ = st[b]
            s_['n'] += 1
            if s_['n'] == 4 and b == NB - 1:
                zs = []
                for c in range(4):
                    zp = jnp.dot(s_['g'][j], w2_v[lo:hi, 128 * c:128 * (c + 1)], preferred_element_type=f32)
                    epilogue(b, s_['z'][:, 128 * c:128 * (c + 1)] + zp, c, c + 1)
                    zs.append(zp)
                return jnp.concatenate(zs, axis=1)
            zp = jnp.dot(s_['g'][j], w2_v[lo:hi, :], preferred_element_type=f32)
            s_['z'] = zp if s_['z'] is None else s_['z'] + zp
            if s_['n'] == 4:
                epilogue(b, s_['z'], 0, 4)
            return zp

        def dur(pc):
            k = pc[0]
            if k == 'q':
                return (pc[4] - pc[3]) * TM
            if k == 'w':
                return 4 * TM
            if k == 'perm':
                return D
            if k == 'm1' or k == 'm2':
                lo, hi = FCH[pc[2]]
                return (hi - lo) // 128 * TM
            return 0

        def run_piece(pc, dl):
            k = pc[0]
            if k == 'q':
                return pQ(pc[1], pc[2], pc[3], pc[4], dl)
            if k == 'w':
                return pW(pc[1])
            if k == 'm1':
                return p1(pc[1], pc[2])
            if k == 'm2':
                return p2(pc[1], pc[2])
            if k == 'perm':
                return perm_part(pc[1])
            if k == 'wait':
                wait(pc[1])
            elif k == 'mods':
                for n in pc[1:]:
                    mod_tile(n)
            return None

        pieces, groups, ix = [], [], {}

        def add(*pcs):
            for pc in pcs:
                ix[pc] = len(pieces)
                pieces.append(pc)

        def grp(fns, a, b_, lat):
            groups.append((fns, ix[a[0]], ix[b_[-1]], lat))

        def run_all():
            NP = len(pieces)
            t0s = []
            t = 0
            for pc in pieces:
                t0s.append(t)
                t += dur(pc)
            t0s.append(t)
            sched = {i: [] for i in range(NP)}
            seen = set()
            dlf = []
            for i, pc in enumerate(pieces):
                d = pc[0] in ('wait', 'w')
                if pc[0] in ('q', 'm1'):
                    if (pc[0], pc[1]) not in seen:
                        d = True
                        seen.add((pc[0], pc[1]))
                    elif pc[0] == 'q' and i + 1 < NP and pieces[i + 1][0] == 'wait':
                        d = True
                dlf.append(d)
            live = [i for i in range(NP) if dur(pieces[i]) > 0]
            live_t = [t0s[i] for i in live]
            seq = 0
            for fns, i0, i1, lat in groups:
                lat = lat + max(dt for dt, _ in fns[0])
                dls = [t0s[i] for i in range(i0 + 1, i1 + 1) if dlf[i]] + [t0s[i1 + 1]]
                slots = []
                for i in range(i0, i1 + 1):
                    if i + 1 < NP and pieces[i + 1][0] == 'wait':
                        continue
                    wt = wa if pieces[i][0] == 'm1' else wb
                    for tt in range(t0s[i], t0s[i + 1], 8):
                        if any(d - lat <= tt < d for d in dls):
                            continue
                        slots.append((tt, wt))
                tot = sum(s_[1] for s_ in slots)
                n = len(fns)
                acc = 0
                kk = 0
                for (tt, wt) in slots:
                    while kk < n and kk / n * tot < acc + wt:
                        for dt, fn in fns[kk]:
                            ii = live[bisect.bisect_right(live_t, tt + dt) - 1]
                            sched[ii].append(((tt + dt - t0s[ii]) / dur(pieces[ii]), seq, fn))
                            seq += 1
                        kk += 1
                    acc += wt
                assert kk == n
            for i, pc in enumerate(pieces):
                arr = run_piece(pc, dlf[i])
                for fr, _, fn in sorted(sched[i], key=lambda t_: (t_[0], t_[1])):
                    ntl = arr.shape[1] // 128 * NT
                    ti = min(int(fr * ntl), ntl - 1)
                    n, r = divmod(ti, NT)
                    fn(arr[8 * r:8 * r + 8, 128 * n:128 * (n + 1)])

        def Qp(b, t, sp=0):
            if sp:
                return [('q', b, t, 0, 4 - sp), ('q', b, t, 4 - sp, 4)]
            return [('q', b, t, 0, 4)]

        def Qs(b, sp=0):
            return Qp(b, 0) + Qp(b, 1) + Qp(b, 2, sp)

        def Wp(b):
            return [('w', b)]

        def Ms(b):
            o = [3, 0, 1, 2] if b == NB - 1 else [0, 1, 2, 3]
            return [('m1', b, o[0]), ('m1', b, o[1]), ('m2', b, o[0]), ('m1', b, o[2]), ('m2', b, o[1]),
                    ('m1', b, o[3]), ('m2', b, o[2]), ('m2', b, o[3])]

        for c in range(4):
            qkb[0][c * KR:c * KR + HALO, :] = jnp.zeros((HALO, 128), f32)
            vb[0][c * KR:c * KR + HALO, :] = jnp.zeros((HALO, 128), f32)
        perm_init()
        wait(0)
        for i in range(len(TIXV)):
            tix[i] = tix2[0, i]
        silu_init()
        for n in range(4, 8):
            mod_tile(n)
        for tk in ln1_fns(0):
            for _, f_ in tk:
                f_(None)

        MODS[('q', 0, 0)] = [[('b', 8)], [('b', 9)], [('b', 10)], [('b', 11)]]
        MODS[('q', 2, 2)] = [[8], [9], [10], [11]]
        MODS[('q', 3, 0)] = [[12], [13], [14], [15]]
        MODS[('q', 3, 1)] = [[16], [17], [18], [19]]
        MODS[('m1', 0, 0)] = [[20], [21], [22], [23]]
        add(('wait', 1), ('perm', 1), *Qp(0, 1))
        add(('wait', 2), ('perm', 2), *Qp(0, 2), *Qp(1, 1), *Qp(1, 2))
        add(('wait', 3), ('mods', 0, 1, 2, 3), ('perm', 0), ('mods', ('b', 4), ('b', 5), ('b', 6), ('b', 7)),
            *Qp(0, 0), *Qp(1, 0), *Qp(2, 0), *Qp(2, 1, 1))
        add(('wait', 4), *Qp(2, 2), *Qs(3), *Wp(0), *Qs(4), *Qs(5, 1))
        add(('wait', 5), *Ms(0))
        add(*Wp(1), *Qs(6), *Ms(1), *Wp(2), *Qs(7))
        for b in (2, 3, 4, 5, 6):
            add(*Wp(b + 1), *Ms(b))
        add(*Ms(7))
        grp(ln1_fns(1), [('perm', 2)], Qp(0, 2), L1h)
        grp(ln1_fns(2), [('perm', 0)], Qp(1, 0), L1a)
        grp([fix_task(t, b, c) for b in range(3) for c in range(4) for t in (1, 2)], Qp(1, 0), Qp(1, 0), LF)
        grp(attn_fns(0, 0), Qp(2, 0), Qp(3, 2), LAa)
        grp(ln1_fns(3), Qp(2, 2), Qp(2, 2), L1h)
        grp([permwo_task(n) for n in range(4)], Qp(3, 0), Qp(3, 2), LP)
        grp(ln1_fns(4), Qp(3, 0), Qp(3, 2), L1)
        grp(attn_fns(1, 0), Wp(0), Qs(5, 1), LAh)
        grp(ln23_fns(0), Qp(4, 0), Qs(5, 1), L23h)
        grp(ln1_fns(5), Qs(4), Qs(4), L1)
        grp(attn_fns(2), Ms(0), Ms(0), LA)
        grp(ln1_fns(6), Ms(0), Wp(1), L1s)
        grp(ln23_fns(1), Qs(6), Qs(6), L23)
        grp(attn_fns(3), Ms(1), Ms(1), LA)
        grp(ln1_fns(7), Ms(1), Wp(2), L1s)
        grp(ln23_fns(2), Qs(7), Wp(3), L23)
        for b in (2, 3, 4, 5, 6):
            grp(ln23_fns(b + 1), Ms(b), Ms(b), L23)
            if b + 2 < NB:
                grp(attn_fns(b + 2), Ms(b), Ms(b), LA)
        run_all()
        for cpy in ocopies:
            cpy.wait()

    def fn(A_x, A_wqkv, A_wo, B_x, B_w1, B_b1, B_w2, B_b2, c, w_mod):
        anyspec = pl.BlockSpec(memory_space=pl.ANY)
        return pl.pallas_call(
            kernel,
            in_specs=[anyspec] * 9,
            out_specs=anyspec,
            out_shape=jax.ShapeDtypeStruct((1, S, D), bf16),
            scratch_shapes=(
                [pltpu.VMEM((TM + 16, D), bf16) for _ in range(NB)]
                + [pltpu.VMEM((NROWS, 128), f32) for _ in range(NB)]
                + [pltpu.VMEM((TM + 8, D), f32) for _ in range(NB)]
                + [pltpu.VMEM((VT + 8, 128), f32) for _ in range(NB)]
                + [pltpu.VMEM((TM, D), bf16) for _ in range(NB - 1)]
                + [pltpu.VMEM((TM, 128), bf16) for _ in range(4)]
                + [pltpu.VMEM((D, D), bf16) for _ in range(3 + 6)]
                + [
                    pltpu.VMEM((D // 2, 3 * D), u32),
                    pltpu.VMEM((D + 16, D), bf16),
                    pltpu.VMEM((4, H * PW + 8, 128), f32),
                    pltpu.VMEM((D // 2, D), u32),
                    pltpu.VMEM((D, F), bf16),
                    pltpu.VMEM((F, D), bf16),
                    pltpu.VMEM((F,), bf16),
                    pltpu.VMEM((D,), bf16),
                    pltpu.VMEM((1, D), bf16),
                    pltpu.VMEM((8, 7 * D), f32),
                    pltpu.VMEM((3 * S // 2, D), u32),
                    pltpu.VMEM((8, F), f32),
                    pltpu.VMEM((16, D), bf16),
                    pltpu.VMEM((16, D), bf16),
                    pltpu.VMEM((16, 3 * D), f32),
                    pltpu.VMEM((4, 128, 128), bf16),
                    pltpu.VMEM((8, 128), jnp.int32),
                    pltpu.SMEM((8, 128), jnp.int32),
                    pltpu.SemaphoreType.DMA((NSEM,)),
                ]),
            compiler_params=pltpu.CompilerParams(
                vmem_limit_bytes=100 * 1024 * 1024,
            ),
        )(A_x, A_wqkv, A_wo, B_w1, B_b1, B_w2, B_b2, c, w_mod)
    return fn


_impl = make()


@jax.jit
def pallas_adaLN_cond__sliding_local_dilated__mixer_channel_mlp__prompt_kernel(
    A_x: jax.Array,
    A_wqkv: jax.Array,
    A_wo: jax.Array,
    B_x: jax.Array,
    B_w1: jax.Array,
    B_b1: jax.Array,
    B_w2: jax.Array,
    B_b2: jax.Array,
    c: jax.Array,
    w_mod: jax.Array,
):
    return _impl(A_x, A_wqkv, A_wo, B_x, B_w1, B_b1, B_w2, B_b2, c, w_mod)
```

```python
import bisect
import functools

import jax
import jax.numpy as jnp
from jax import lax
import jax.experimental.pallas as pl
import jax.experimental.pallas.tpu as pltpu

S, D, F = 2048, 512, 1792
H, DH, W, DIL = 32, 16, 8, 2
HALO = 16
LOG2E = 1.4426950408889634
EPS = 1e-5
GC0 = 0.7978845608028654
GC1 = 0.7978845608028654 * 0.044715
f32 = jnp.float32
bf16 = jnp.bfloat16
u32 = jnp.uint32
P = functools.partial


def _ln(x):
    m = jnp.mean(x, axis=-1, keepdims=True)
    xc = x - m
    v = jnp.mean(xc * xc, axis=-1, keepdims=True)
    return xc * jnp.exp2(-0.5 * jnp.log2(v + EPS))


def _mul8(x, r8):
    R, N = x.shape
    return (x.reshape(R // 8, 8, N) * r8.reshape(1, 8, N)).reshape(R, N)


def _add8(x, r8):
    R, N = x.shape
    return (x.reshape(R // 8, 8, N) + r8.reshape(1, 8, N)).reshape(R, N)


def _pk(x):
    return pltpu.bitcast(x, u32)


def _upk(x):
    return pltpu.bitcast(x, bf16)


def make(RC=8, LC=32, L1C=32, wa=10, wb=25, LA=250, L23=150, sa=16, T=250, sb=28,
         DA=450, LAh=250, LP=500, L1h=50, PW=17, D1a=450, L1a=450, D1h=350, D1s=500, L1=300, L1s=300,
         D23h=650, D23s=800, L23h=150, LAa=250, LF=50, kp=8, qp=8):
    TM = 256
    NB = S // TM
    KE = TM + HALO
    KR = KE + kp
    QR = TM + qp
    QB = 4 * KR
    VT = 4 * KR
    TB = QB + 4 * QR
    NROWS = TB + 8
    NT = TM // 8
    FCH = [(0, 512), (512, 1024), (1024, 1536), (1536, 1792)]
    WGROUPS = [('c', 'x0', 'wca', 'tix'), ('wk',), ('wv', 'x1'), ('wsa', 'wq', 'x2'),
               ('x3', 'wo', 'wga', 'wsb', 'wcb', 'x4', 'x5'), ('b1', 'w1', 'w2', 'wgb', 'b2', 'x6', 'x7')]
    SID = {n: i for i, g_ in enumerate(WGROUPS) for n in g_}
    NSEM = len(WGROUPS) + 1

    def kernel(x_hbm, wqkv_hbm, wo_hbm, w1_hbm, b1_hbm, w2_hbm, b2_hbm, c_hbm, wmod_hbm, out_hbm, *scr):
        scr = list(scr)
        xb = [scr.pop(0) for _ in range(NB)]
        qkb = [scr.pop(0) for _ in range(NB)]
        x1b = [scr.pop(0) for _ in range(NB)]
        vb = [scr.pop(0) for _ in range(NB)]
        outb = [scr.pop(0) for _ in range(NB - 1)]
        outl = [scr.pop(0) for _ in range(4)]
        wraw = [scr.pop(0) for _ in range(3)]
        wmodb = [scr.pop(0) for _ in range(6)]
        (wqkv_p, wo_v, wo_f, wo_p, w1_v, w2_v, b1_v, b2_v, c_v,
         mod_ref, ha_v, b1_f, sc_v, sa_v, bias_v, qm_v, tix_v, tix2, sems) = scr

        ocopies = []

        def ocopy(src, b, c0, c1):
            cpy = pltpu.make_async_copy(src, out_hbm.at[0, pl.ds(b * TM, TM), pl.ds(128 * c0, 128 * (c1 - c0))],
                                        sems.at[NSEM - 1])
            ocopies.append(cpy)
            cpy.start()

        def mk(name, src, dst):
            return pltpu.make_async_copy(src, dst, sems.at[SID[name]])

        def wm(i, name):
            return mk(name, wmod_hbm.at[:, i * D:(i + 1) * D], wmodb[i])

        cp = dict(
            c=mk('c', c_hbm, c_v),
            wq=mk('wq', wqkv_hbm.at[:, 0:D], wraw[0]),
            wk=mk('wk', wqkv_hbm.at[:, D:2 * D], wraw[1]),
            wv=mk('wv', wqkv_hbm.at[:, 2 * D:3 * D], wraw[2]),
            wsa=wm(0, 'wsa'), wca=wm(1, 'wca'), wga=wm(2, 'wga'), wsb=wm(3, 'wsb'), wcb=wm(4, 'wcb'), wgb=wm(5, 'wgb'),
            wo=mk('wo', wo_hbm, wo_v.at[pl.ds(0, D), :]),
            w1=mk('w1', w1_hbm, w1_v), w2=mk('w2', w2_hbm, w2_v),
            b1=mk('b1', b1_hbm, b1_v), b2=mk('b2', b2_hbm, b2_v),
            tix=mk('tix', tix_v, tix2),
        )
        for b in range(NB):
            cp['x%d' % b] = mk('x%d' % b, x_hbm.at[0, pl.ds(b * TM, TM), :], xb[b].at[pl.ds(0, TM), :])
        for g_ in WGROUPS:
            for o in g_:
                if o != 'tix':
                    cp[o].start()

        def wait(gi):
            for n in WGROUPS[gi]:
                cp[n].wait()

        TIXV = [TB, TM, 0, D, VT, 8]
        lane0 = lax.broadcasted_iota(jnp.int32, (8, 128), 1)
        tv = jnp.zeros((8, 128), jnp.int32)
        for i, v_ in enumerate(TIXV):
            tv = jnp.where(lane0 == i, v_, tv)
        tix_v[...] = tv
        cp['tix'].start()
        tix = [None] * len(TIXV)

        def silu_init():
            c = c_v[...].astype(f32)
            sc = c * jax.nn.sigmoid(c)
            sc_v[...] = jnp.broadcast_to(sc, (16, D)).astype(bf16)

        def mod_tile(n):
            if isinstance(n, tuple):
                nn = n[1]
                bias_v[0:8, 128 * nn:128 * (nn + 1)] = jnp.dot(sa_v[0:8, :], _upk(wqkv_p[:, 128 * nn:128 * (nn + 1)]),
                                                               preferred_element_type=f32)
                return
            cs = slice(128 * n, 128 * (n + 1))
            m = jnp.dot(sc_v[0:8, :], wmodb[n // 4][:, 128 * (n % 4):128 * (n % 4 + 1)], preferred_element_type=f32)
            if 4 <= n < 8 or 16 <= n < 20:
                m = 1.0 + m
            if n < 4:
                sa_v[:, cs] = jnp.concatenate([m, m], axis=0).astype(bf16)
            if n >= 20:
                b2 = b2_v[...].astype(f32).reshape(1, D)[:, 128 * (n - 20):128 * (n - 19)]
                mod_ref[:, 128 * (n + 4):128 * (n + 5)] = m * b2
                m = 0.5 * m
            mod_ref[:, cs] = m

        def modv(i):
            return mod_ref[:, i * D:(i + 1) * D]

        def perm_init():
            r = lax.broadcasted_iota(jnp.int32, (128, 128), 0)
            cc = lax.broadcasted_iota(jnp.int32, (128, 128), 1)
            for cpi in range(4):
                tgt = ((r & 3) << 5) | (((cpi ^ ((r >> 2) & 3))) << 3) | (r >> 4)
                qm_v[cpi] = jnp.where(cc == tgt, 1.0, 0.0).astype(bf16)

        def perm_part(t):
            lane = lax.broadcasted_iota(jnp.int32, (D // 2, 128), 1)
            e0 = (lane & 4) != 0
            e1 = (lane & 8) != 0
            ch = [pltpu.bitcast(wraw[t][:, 128 * c:128 * (c + 1)], u32) for c in range(4)]
            res = None
            for cpi in range(4):
                lo_ = jnp.where(e0, ch[cpi ^ 1], ch[cpi ^ 0])
                hi_ = jnp.where(e0, ch[cpi ^ 3], ch[cpi ^ 2])
                mg = pltpu.bitcast(jnp.where(e1, hi_, lo_), bf16)
                rr = jnp.dot(mg, qm_v[cpi], preferred_element_type=f32)
                if cpi == 0:
                    res = rr
                wqkv_p[:, t * D + 128 * cpi:t * D + 128 * (cpi + 1)] = _pk(rr.astype(bf16))
            return jnp.concatenate([res[0:TM, :], res[TM:2 * TM, :]], axis=1)

        def dynrows(r, n):
            return pl.ds(pl.multiple_of(tix[2] + r // 2, 8), n // 2)

        def tok16(tokv):
            return jnp.concatenate([tokv, tokv], axis=0).astype(bf16)

        def permwo_task(n):
            def sA(tokv):
                wo_v[pl.ds(pl.multiple_of(tix[3], 16), 16), 0:128] = tok16(tokv)
                wf = wo_v[0:D, 128 * n:128 * (n + 1)].astype(f32)
                for hh in range(H):
                    wo_f[n, pl.ds(hh * PW, 16), :] = wf[16 * hh:16 * hh + 16, :]
                for cpi in range(4):
                    for t in range(4):
                        parts = []
                        for g in range(4):
                            d = ((cpi ^ g) << 2) | t
                            parts.append(wo_f[n, pl.ds(g * 8 * PW + d, 8, stride=PW), :])
                        wo_p[cpi * 64 + t * 16:cpi * 64 + t * 16 + 16, 128 * n:128 * (n + 1)] = _pk(
                            jnp.concatenate(parts, axis=0).astype(bf16))
            return [(0, sA)]

        def ln1_task(b, j):
            r0 = j * L1C
            stt = {}

            def sA(tokv):
                if tokv is not None:
                    xb[b][pl.ds(pl.multiple_of(tix[1], 16), 16), 0:128] = tok16(tokv)
                x = xb[b][r0:r0 + L1C, :].astype(f32)
                hh = _mul8(_ln(x), modv(1))
                if b >= 2:
                    hh = _add8(hh, modv(0))
                stt['h'] = _pk(hh.astype(bf16))

            def sB(tokv):
                ha_v[dynrows(S + b * TM + r0, L1C), :] = stt['h']

            return [(0, sA), (D1a if b == 2 else (D1h if b < 6 else D1s), sB)]

        def ln23_task(b, j):
            r0 = j * LC
            stt = {}

            def sA(tokv):
                x1b[b][pl.ds(pl.multiple_of(tix[1], 8), 8), 0:128] = tokv
                h2 = _add8(_mul8(_ln(x1b[b][r0:r0 + LC, :]), modv(4)), modv(3))
                stt['y'] = _pk(_ln(h2).astype(bf16))

            def sB(tokv):
                ha_v[dynrows(2 * S + b * TM + r0, LC), :] = stt['y']

            return [(0, sA), (D23h if b == 0 else D23s, sB)]

        attprev = {}

        def attn_task(b, j, micro):
            r0 = j * RC
            qk = qkb[b]
            stt = dict(logits=[], outs=[])

            def qk_step(w, tokv):
                if tokv is not None:
                    qk[pl.ds(pl.multiple_of(tix[0], 8), 8), :] = tokv
                if w == 0:
                    stt['q'] = [qk[QB + c * QR + r0:QB + c * QR + r0 + RC, :] for c in range(4)]
                q = stt['q']
                off = HALO + r0 - DIL * w
                ps_ = [q[c] * qk[pl.ds(c * KR + off, RC), :] for c in range(4)]
                acc = (ps_[0] + ps_[1]) + (ps_[2] + ps_[3])
                if micro:
                    acc = (acc + pltpu.roll(acc, 64, 1)) + (pltpu.roll(acc, 32, 1) + pltpu.roll(acc, 96, 1))
                else:
                    acc = acc + pltpu.roll(acc, 64, 1)
                    acc = acc + pltpu.roll(acc, 32, 1)
                if b == 0 and r0 < DIL * w:
                    row = r0 + lax.broadcasted_iota(jnp.int32, (RC, 128), 0)
                    acc = jnp.where(row >= DIL * w, acc, -1e9 * LOG2E)
                stt['logits'].append(acc)
                if w == W - 1:
                    lg = stt['logits']
                    m = jnp.maximum(jnp.maximum(jnp.maximum(lg[0], lg[1]), jnp.maximum(lg[2], lg[3])),
                                    jnp.maximum(jnp.maximum(lg[4], lg[5]), jnp.maximum(lg[6], lg[7])))
                    ps = [jnp.exp2(l - m) for l in lg]
                    den = ((ps[0] + ps[1]) + (ps[2] + ps[3])) + ((ps[4] + ps[5]) + (ps[6] + ps[7]))
                    r_ = pl.reciprocal(den, approx=True)
                    stt['inv'] = r_ * (2.0 - den * r_)
                    stt['ps'] = ps

            def pv_step(c, tokv):
                if tokv is not None:
                    vb[b][pl.ds(pl.multiple_of(tix[4], 8), 8), :] = tokv
                ps = stt['ps']
                ts = [ps[w] * vb[b][pl.ds(c * KR + HALO + r0 - DIL * w, RC), :] for w in range(W)]
                acc = ((ts[0] + ts[1]) + (ts[2] + ts[3])) + ((ts[4] + ts[5]) + (ts[6] + ts[7]))
                stt['outs'].append(acc * stt['inv'])
                if c == 3:
                    o = jnp.concatenate(stt['outs'], axis=1)
                    if j % 2 == 0:
                        attprev[b] = o
                    else:
                        oo = jnp.concatenate([attprev[b], o], axis=0).astype(bf16)
                        ha_v[dynrows(b * TM + r0 - RC, 2 * RC), :] = _pk(oo)

            if micro:
                return [(sa * w, P(qk_step, w)) for w in range(W)] + [(T + sb * c, P(pv_step, c)) for c in range(4)]

            def allA(tokv):
                qk_step(0, tokv)
                for w in range(1, W):
                    qk_step(w, None)
                for c in range(3):
                    pv_step(c, None)

            def allB(tokv):
                pv_step(3, None)
            return [(0, allA), (DA, allB)]

        def fix_task(t, b, c):
            def sA(tokv):
                ref = qkb[b] if t == 1 else vb[b]
                bias_v[pl.ds(pl.multiple_of(tix[5], 8), 8), 0:128] = tokv
                lo = c * KR + (HALO if b == 0 else 0)
                hi = c * KR + (HALO if b == 2 else KE)
                ref[lo:hi, :] = _add8(ref[lo:hi, :], bias_v[0:8, t * D + 128 * c:t * D + 128 * (c + 1)])
            return [(0, sA)]

        def attn_fns(b, mi=1):
            return [attn_task(b, j, mi) for j in range(TM // RC)]

        def ln1_fns(b):
            return [ln1_task(b, j) for j in range(TM // L1C)]

        def ln23_fns(b):
            return [ln23_task(b, j) for j in range(TM // LC)]

        hs = {}
        st = {}
        MODS = {}

        def dot_mods(lhs_, wget, c0, ncol, mods):
            if not mods:
                return jnp.dot(lhs_, wget(c0, c0 + ncol), preferred_element_type=f32)
            outs = []
            for c in range(ncol // 128):
                outs.append(jnp.dot(lhs_, wget(c0 + 128 * c, c0 + 128 * (c + 1)), preferred_element_type=f32))
                for n in mods[c]:
                    mod_tile(n)
            return jnp.concatenate(outs, axis=1)

        def pQ(b, t, c0, c1, dl):
            if dl or b not in hs:
                hs[b] = _upk(ha_v[(S + b * TM) // 2:(S + (b + 1) * TM) // 2, :])
            lhs_ = hs[b]
            pig = b == 0 and t == 0
            if pig:
                lhs_ = jnp.concatenate([sa_v[...], lhs_], axis=0)
            mods = MODS.get(('q', b, t))
            r = dot_mods(lhs_, lambda lo_, hi_: _upk(wqkv_p[:, lo_:hi_]), t * D + 128 * c0, 128 * (c1 - c0), mods[c0:c1] if mods else None)
            if pig:
                bq = r[0:8, :]
                bias_v[0:8, 128 * c0:128 * c1] = bq
                r = r[16:, :]
            elif b == 1 and t == 0:
                bq = bias_v[0:8, 128 * c0:128 * c1]
            for c in range(c0, c1):
                rc = r[:, 128 * (c - c0):128 * (c - c0 + 1)]
                if t == 0:
                    if b < 2:
                        rc = _add8(rc, bq[:, 128 * (c - c0):128 * (c - c0 + 1)])
                    qkb[b][QB + c * QR:QB + c * QR + TM, :] = rc * (DH ** -0.5 * LOG2E)
                else:
                    bufs = qkb if t == 1 else vb
                    bufs[b][c * KR + HALO:c * KR + KE, :] = rc
                    if b + 1 < NB:
                        bufs[b + 1][c * KR:c * KR + HALO, :] = rc[TM - HALO:TM, :]
            return r

        def pW(b):
            a = jnp.dot(_upk(ha_v[b * TM // 2:(b + 1) * TM // 2, :]), _upk(wo_p[...]), preferred_element_type=f32)
            x1b[b][0:TM, :] = xb[b][0:TM, :].astype(f32) + _mul8(a, modv(2))
            return a

        def p1(b, j):
            if b not in st:
                st[b] = dict(y=_upk(ha_v[(2 * S + b * TM) // 2:(2 * S + (b + 1) * TM) // 2, :]), g={}, z=None, n=0)
            lo, hi = FCH[j]
            if b == 0 and j == 0:
                b1_f[...] = jnp.broadcast_to(b1_v[...].astype(f32).reshape(1, F), (8, F))
            u = _add8(dot_mods(st[b]['y'], lambda lo_, hi_: w1_v[:, lo_:hi_], lo, hi - lo, MODS.get(('m1', b, j))), b1_f[:, lo:hi])
            t = jnp.tanh(u * (GC0 + GC1 * (u * u)))
            st[b]['g'][j] = (u + u * t).astype(bf16)
            return u

        def epilogue(b, z, c0, c1):
            cs = slice(128 * c0, 128 * c1)
            hg = mod_ref[:, 5 * D + 128 * c0:5 * D + 128 * c1]
            gb2 = mod_ref[:, 6 * D + 128 * c0:6 * D + 128 * c1]
            dst = outl[c0] if b == NB - 1 else outb[b]
            dst[...] = (_add8(x1b[b][0:TM, cs], gb2) + _mul8(z, hg)).astype(bf16)
            ocopy(dst, b, c0, c1)

        def p2(b, j):
            lo, hi = FCH[j]
            s_ = st[b]
            s_['n'] += 1
            if s_['n'] == 4 and b == NB - 1:
                zs = []
                for c in range(4):
                    zp = jnp.dot(s_['g'][j], w2_v[lo:hi, 128 * c:128 * (c + 1)], preferred_element_type=f32)
                    epilogue(b, s_['z'][:, 128 * c:128 * (c + 1)] + zp, c, c + 1)
                    zs.append(zp)
                return jnp.concatenate(zs, axis=1)
            zp = jnp.dot(s_['g'][j], w2_v[lo:hi, :], preferred_element_type=f32)
            s_['z'] = zp if s_['z'] is None else s_['z'] + zp
            if s_['n'] == 4:
                epilogue(b, s_['z'], 0, 4)
            return zp

        def dur(pc):
            k = pc[0]
            if k == 'q':
                return (pc[4] - pc[3]) * TM
            if k == 'w':
                return 4 * TM
            if k == 'perm':
                return D
            if k == 'm1' or k == 'm2':
                lo, hi = FCH[pc[2]]
                return (hi - lo) // 128 * TM
            return 0

        def run_piece(pc, dl):
            k = pc[0]
            if k == 'q':
                return pQ(pc[1], pc[2], pc[3], pc[4], dl)
            if k == 'w':
                return pW(pc[1])
            if k == 'm1':
                return p1(pc[1], pc[2])
            if k == 'm2':
                return p2(pc[1], pc[2])
            if k == 'perm':
                return perm_part(pc[1])
            if k == 'wait':
                wait(pc[1])
            elif k == 'mods':
                for n in pc[1:]:
                    mod_tile(n)
            return None

        pieces, groups, ix = [], [], {}

        def add(*pcs):
            for pc in pcs:
                ix[pc] = len(pieces)
                pieces.append(pc)

        def grp(fns, a, b_, lat):
            groups.append((fns, ix[a[0]], ix[b_[-1]], lat))

        def run_all():
            NP = len(pieces)
            t0s = []
            t = 0
            for pc in pieces:
                t0s.append(t)
                t += dur(pc)
            t0s.append(t)
            sched = {i: [] for i in range(NP)}
            seen = set()
            dlf = []
            for i, pc in enumerate(pieces):
                d = pc[0] in ('wait', 'w')
                if pc[0] in ('q', 'm1'):
                    if (pc[0], pc[1]) not in seen:
                        d = True
                        seen.add((pc[0], pc[1]))
                    elif pc[0] == 'q' and i + 1 < NP and pieces[i + 1][0] == 'wait':
                        d = True
                dlf.append(d)
            live = [i for i in range(NP) if dur(pieces[i]) > 0]
            live_t = [t0s[i] for i in live]
            seq = 0
            for fns, i0, i1, lat in groups:
                lat = lat + max(dt for dt, _ in fns[0])
                dls = [t0s[i] for i in range(i0 + 1, i1 + 1) if dlf[i]] + [t0s[i1 + 1]]
                slots = []
                for i in range(i0, i1 + 1):
                    if i + 1 < NP and pieces[i + 1][0] == 'wait':
                        continue
                    wt = wa if pieces[i][0] == 'm1' else wb
                    for tt in range(t0s[i], t0s[i + 1], 8):
                        if any(d - lat <= tt < d for d in dls):
                            continue
                        slots.append((tt, wt))
                tot = sum(s_[1] for s_ in slots)
                n = len(fns)
                acc = 0
                kk = 0
                for (tt, wt) in slots:
                    while kk < n and kk / n * tot < acc + wt:
                        for dt, fn in fns[kk]:
                            ii = live[bisect.bisect_right(live_t, tt + dt) - 1]
                            sched[ii].append(((tt + dt - t0s[ii]) / dur(pieces[ii]), seq, fn))
                            seq += 1
                        kk += 1
                    acc += wt
                assert kk == n
            for i, pc in enumerate(pieces):
                arr = run_piece(pc, dlf[i])
                for fr, _, fn in sorted(sched[i], key=lambda t_: (t_[0], t_[1])):
                    ntl = arr.shape[1] // 128 * NT
                    ti = min(int(fr * ntl), ntl - 1)
                    n, r = divmod(ti, NT)
                    fn(arr[8 * r:8 * r + 8, 128 * n:128 * (n + 1)])

        def Qp(b, t, sp=0):
            if sp:
                return [('q', b, t, 0, 4 - sp), ('q', b, t, 4 - sp, 4)]
            return [('q', b, t, 0, 4)]

        def Qs(b, sp=0):
            return Qp(b, 0) + Qp(b, 1) + Qp(b, 2, sp)

        def Wp(b):
            return [('w', b)]

        def Ms(b):
            o = [3, 0, 1, 2] if b == NB - 1 else [0, 1, 2, 3]
            return [('m1', b, o[0]), ('m1', b, o[1]), ('m2', b, o[0]), ('m1', b, o[2]), ('m2', b, o[1]),
                    ('m1', b, o[3]), ('m2', b, o[2]), ('m2', b, o[3])]

        for c in range(4):
            qkb[0][c * KR:c * KR + HALO, :] = jnp.zeros((HALO, 128), f32)
            vb[0][c * KR:c * KR + HALO, :] = jnp.zeros((HALO, 128), f32)
        perm_init()
        wait(0)
        for i in range(len(TIXV)):
            tix[i] = tix2[0, i]
        silu_init()
        for n in range(4, 8):
            mod_tile(n)
        for tk in ln1_fns(0):
            for _, f_ in tk:
                f_(None)

        MODS[('q', 0, 0)] = [[('b', 8)], [('b', 9)], [('b', 10)], [('b', 11)]]
        MODS[('q', 2, 2)] = [[8], [9], [10], [11]]
        MODS[('q', 3, 0)] = [[12], [13], [14], [15]]
        MODS[('q', 3, 1)] = [[16], [17], [18], [19]]
        MODS[('m1', 0, 0)] = [[20], [21], [22], [23]]
        add(('wait', 1), ('perm', 1), *Qp(0, 1))
        add(('wait', 2), ('perm', 2), *Qp(0, 2), *Qp(1, 1), *Qp(1, 2))
        add(('wait', 3), ('mods', 0, 1, 2, 3), ('perm', 0), ('mods', ('b', 4), ('b', 5), ('b', 6), ('b', 7)),
            *Qp(0, 0), *Qp(1, 0), *Qp(2, 0), *Qp(2, 1, 1))
        add(('wait', 4), *Qp(2, 2), *Qs(3), *Wp(0), *Qs(4), *Qs(5, 1))
        add(('wait', 5), *Ms(0))
        add(*Wp(1), *Qs(6), *Ms(1), *Wp(2), *Qs(7))
        for b in (2, 3, 4, 5, 6):
            add(*Wp(b + 1), *Ms(b))
        add(*Ms(7))
        grp(ln1_fns(1), [('perm', 2)], Qp(0, 2), L1h)
        grp(ln1_fns(2), [('perm', 0)], Qp(1, 0), L1a)
        grp([fix_task(t, b, c) for b in range(3) for c in range(4) for t in (1, 2)], Qp(1, 0), Qp(1, 0), LF)
        grp(attn_fns(0, 0), Qp(2, 0), Qp(3, 2), LAa)
        grp(ln1_fns(3), Qp(2, 2), Qp(2, 2), L1h)
        grp([permwo_task(n) for n in range(4)], Qp(3, 0), Qp(3, 2), LP)
        grp(ln1_fns(4), Qp(3, 0), Qp(3, 2), L1)
        grp(attn_fns(1, 0), Wp(0), Qs(5, 1), LAh)
        grp(ln23_fns(0), Qp(4, 0), Qs(5, 1), L23h)
        grp(ln1_fns(5), Qs(4), Qs(4), L1)
        grp(attn_fns(2), Ms(0), Ms(0), LA)
        grp(ln1_fns(6), Ms(0), Wp(1), L1s)
        grp(ln23_fns(1), Qs(6), Qs(6), L23)
        grp(attn_fns(3), Ms(1), Ms(1), LA)
        grp(ln1_fns(7), Ms(1), Wp(2), L1s)
        grp(ln23_fns(2), Qs(7), Wp(3), L23)
        for b in (2, 3, 4, 5, 6):
            grp(ln23_fns(b + 1), Ms(b), Ms(b), L23)
            if b + 2 < NB:
                grp(attn_fns(b + 2), Ms(b), Ms(b), LA)
        run_all()
        for cpy in ocopies:
            cpy.wait()

    def fn(A_x, A_wqkv, A_wo, B_x, B_w1, B_b1, B_w2, B_b2, c, w_mod):
        anyspec = pl.BlockSpec(memory_space=pl.ANY)
        return pl.pallas_call(
            kernel,
            in_specs=[anyspec] * 9,
            out_specs=anyspec,
            out_shape=jax.ShapeDtypeStruct((1, S, D), bf16),
            scratch_shapes=(
                [pltpu.VMEM((TM + 16, D), bf16) for _ in range(NB)]
                + [pltpu.VMEM((NROWS, 128), f32) for _ in range(NB)]
                + [pltpu.VMEM((TM + 8, D), f32) for _ in range(NB)]
                + [pltpu.VMEM((VT + 8, 128), f32) for _ in range(NB)]
                + [pltpu.VMEM((TM, D), bf16) for _ in range(NB - 1)]
                + [pltpu.VMEM((TM, 128), bf16) for _ in range(4)]
                + [pltpu.VMEM((D, D), bf16) for _ in range(3 + 6)]
                + [
                    pltpu.VMEM((D // 2, 3 * D), u32),
                    pltpu.VMEM((D + 16, D), bf16),
                    pltpu.VMEM((4, H * PW + 8, 128), f32),
                    pltpu.VMEM((D // 2, D), u32),
                    pltpu.VMEM((D, F), bf16),
                    pltpu.VMEM((F, D), bf16),
                    pltpu.VMEM((F,), bf16),
                    pltpu.VMEM((D,), bf16),
                    pltpu.VMEM((1, D), bf16),
                    pltpu.VMEM((8, 7 * D), f32),
                    pltpu.VMEM((3 * S // 2, D), u32),
                    pltpu.VMEM((8, F), f32),
                    pltpu.VMEM((16, D), bf16),
                    pltpu.VMEM((16, D), bf16),
                    pltpu.VMEM((16, 3 * D), f32),
                    pltpu.VMEM((4, 128, 128), bf16),
                    pltpu.VMEM((8, 128), jnp.int32),
                    pltpu.SMEM((8, 128), jnp.int32),
                    pltpu.SemaphoreType.DMA((NSEM,)),
                ]),
            compiler_params=pltpu.CompilerParams(
                vmem_limit_bytes=100 * 1024 * 1024,
            ),
        )(A_x, A_wqkv, A_wo, B_w1, B_b1, B_w2, B_b2, c, w_mod)
    return fn


_impl = make()


@jax.jit
def pallas_adaLN_cond__sliding_local_dilated__mixer_channel_mlp__prompt_kernel(
    A_x: jax.Array,
    A_wqkv: jax.Array,
    A_wo: jax.Array,
    B_x: jax.Array,
    B_w1: jax.Array,
    B_b1: jax.Array,
    B_w2: jax.Array,
    B_b2: jax.Array,
    c: jax.Array,
    w_mod: jax.Array,
):
    return _impl(A_x, A_wqkv, A_wo, B_x, B_w1, B_b1, B_w2, B_b2, c, w_mod)
```
